```python
import os as _os
_os.environ.setdefault('JAX_PLATFORMS', 'cpu')
import jax
import jax.numpy as jnp

def _softmax(x, axis=-1):
    return jax.nn.softmax(x, axis=axis)

def _gelu(x):
    return jax.nn.gelu(x, approximate=True)

def _silu(x):
    return jax.nn.silu(x)

def _sigmoid(x):
    return jax.nn.sigmoid(x)

def _layernorm(x, axis=-1, eps=1e-05):
    m = jnp.mean(x, axis=axis, keepdims=True)
    v = jnp.var(x, axis=axis, keepdims=True)
    return (x - m) / jnp.sqrt(v + eps)

def _scatter_add(tgt, idx, src, axis=0):
    return tgt.at[idx].add(src)

def _segment_sum(src, seg, n):
    return jax.ops.segment_sum(src, seg, n)

class _Rng:

    def __init__(self, key):
        self._k = key

    def _next(self):
        self._k, sub = jax.random.split(self._k)
        return sub

    def normal(self, shape):
        return jax.random.normal(self._next(), shape, dtype=jnp.bfloat16)

    def randint(self, lo, hi, shape):
        return jax.random.randint(self._next(), shape, lo, hi, dtype=jnp.int32)

    def uniform(self, shape, lo=0.0, hi=1.0):
        return jax.random.uniform(self._next(), shape, jnp.bfloat16, lo, hi)

    def permutation(self, n):
        return jax.random.permutation(self._next(), n)
kernel_name = 'adaLN_cond__grouped_kv_mqa__mixer_gmlp__prompt'

def setup_inputs():
    _rng = _Rng(jax.random.key(int.from_bytes(__import__("os").urandom(4), "little")))
    _w = lambda a: (lambda t: t.astype(jnp.bfloat16) if jnp.issubdtype(t.dtype, jnp.floating) else t)(jnp.asarray(a))

    def _A_setup():
        B, S, D, H = (1, 2048, 512, 32)
        Dh = D // H
        return {'x': _w((lambda *s: _rng.normal(s) * 0.05)(B, S, D)), 'wq': _w((lambda *s: _rng.normal(s) * 0.05)(D, H * Dh)), 'wk': _w((lambda *s: _rng.normal(s) * 0.05)(D, Dh)), 'wv': _w((lambda *s: _rng.normal(s) * 0.05)(D, Dh)), 'wo': _w((lambda *s: _rng.normal(s) * 0.05)(H * Dh, D))}
    _A_in = _A_setup()

    def _B_setup():
        B, S, D, F = (1, 2048, 512, 1792)
        Fh = F // 2
        return {'x': _w((lambda *s: _rng.normal(s) * 0.05)(B, S, D)), 'w_in': _w((lambda *s: _rng.normal(s) * 0.4)(D, 2 * Fh)), 'w_sp': _w(0.01 * (lambda *s: _rng.normal(s) * 0.4)(S, S)), 'b_sp': _w(1.0 + 0.01 * (lambda *s: _rng.normal(s) * 0.05)(S)), 'w_out': _w((lambda *s: _rng.normal(s) * 0.05)(Fh, D))}
    _B_in = _B_setup()
    return {'A_x': _A_in['x'], 'A_wq': _A_in['wq'], 'A_wk': _A_in['wk'], 'A_wv': _A_in['wv'], 'A_wo': _A_in['wo'], 'B_x': _B_in['x'], 'B_w_in': _B_in['w_in'], 'B_w_sp': _B_in['w_sp'], 'B_b_sp': _B_in['b_sp'], 'B_w_out': _B_in['w_out'], 'c': _w((lambda *s: _rng.normal(s) * 0.05)(1, 512) * 8.0), 'w_mod': _w((lambda *s: _rng.normal(s) * 0.05)(512, 6 * 512) * 512 ** (-0.5) * 8.0)}

def reference(A_x, A_wq, A_wk, A_wv, A_wo, B_x, B_w_in, B_w_sp, B_b_sp, B_w_out, c, w_mod):

    def _A_ref(x, wq, wk, wv, wo):
        B, S, D = x.shape
        H = 32
        Dh = D // H
        q = (lambda x, *d: x.transpose(*d))((x @ wq).reshape(B, S, H, Dh), 0, 2, 1, 3)
        k = x @ wk
        v = x @ wv
        scores = jnp.einsum('bhqd,bkd->bhqk', q, k) * Dh ** (-0.5)
        p = _softmax(scores, axis=-1)
        o = jnp.einsum('bhqk,bkd->bhqd', p, v)
        return (lambda x, *d: x.transpose(*d))(o, 0, 2, 1, 3).reshape(B, S, H * Dh) @ wo

    def _B_ref(x, w_in, w_sp, b_sp, w_out):
        B, S, D = x.shape
        F = w_in.shape[-1]
        Fh = F // 2
        z = _gelu(jnp.einsum('bsd,df->bsf', x, w_in))
        z1 = z[..., :Fh].copy()
        z2 = _layernorm(z[..., Fh:], axis=-1)
        g = jnp.einsum('ts,bsf->btf', w_sp, z2) + b_sp[None, :, None]
        return jnp.einsum('bsf,fd->bsd', z1 * g, w_out)
    x = A_x
    mod = (_silu(c) @ w_mod).reshape(c.shape[0], 6, 1, -1)
    sa, ca, ga, sb, cb, gb = (mod[:, 0].copy(), mod[:, 1].copy(), mod[:, 2].copy(), mod[:, 3].copy(), mod[:, 4].copy(), mod[:, 5].copy())
    h = _layernorm(x, axis=-1) * (1 + ca) + sa
    x = x + ga * _A_ref(h, A_wq, A_wk, A_wv, A_wo)
    h = _layernorm(x, axis=-1) * (1 + cb) + sb
    x = x + gb * _B_ref(h, B_w_in, B_w_sp, B_b_sp, B_w_out)
    return x
```

```python
import functools
import math

import jax
import jax.numpy as jnp
from jax import lax
import jax.experimental.pallas as pl
import jax.experimental.pallas.tpu as pltpu

F32 = jnp.float32
BF16 = jnp.bfloat16
EPS = 1e-5
LOG2E = 1.4426950408889634


def _ln(x):
    m = jnp.mean(x, axis=-1, keepdims=True)
    xc = x - m
    v = jnp.mean(xc * xc, axis=-1, keepdims=True)
    return xc * lax.rsqrt(v + EPS)


def _gelu_tanh(x):
    c0 = math.sqrt(2.0 / math.pi)
    inner = x * (c0 + (c0 * 0.044715) * (x * x))
    hx = 0.5 * x
    return hx + hx * jnp.tanh(inner)


def _kernel(x_hbm, wq_hbm, wk_ref, wv_ref, wo_hbm, win_hbm, wsp_hbm, bsp_ref,
            wout_hbm, c_ref, wmod_hbm, out_hbm,
            x_v, wq_v, wo_v, win_v, wsp_v, wout_v, wmod_v,
            wT_v, qT_v, k_v, vT_v, sA_v, sB_v, oT_v, x1_v, z1_v, z2_v, mod_v,
            out_v, sems, osems,
            *, S, D, H, DH, FH, TQ, TK, TB, TR):
    NQ = S // TQ
    NC = S // TK
    NB = S // TB
    NR = S // TR

    def cp(src, dst, i):
        return pltpu.make_async_copy(src, dst, sems.at[i])

    cp_modA = cp(wmod_hbm.at[:, pl.ds(0, 2 * D)], wmod_v.at[:, pl.ds(0, 2 * D)], 0)
    cp_wq = cp(wq_hbm, wq_v, 1)
    cp_x = [cp(x_hbm.at[pl.ds(b * TB, TB), :], x_v.at[pl.ds(b * TB, TB), :], 2 + b)
            for b in range(NB)]
    base = 2 + NB
    cp_modB = cp(wmod_hbm.at[:, pl.ds(2 * D, 4 * D)], wmod_v.at[:, pl.ds(2 * D, 4 * D)], base)
    cp_wo = cp(wo_hbm, wo_v, base + 1)
    cp_win = cp(win_hbm, win_v, base + 2)
    cp_wout = cp(wout_hbm, wout_v, base + 3)
    cp_wsp = cp(wsp_hbm, wsp_v, base + 4)

    cp_modA.start()
    cp_wq.start()
    for b in range(NB):
        cp_x[b].start()

    cvec = c_ref[...].astype(F32)
    sc = cvec * (1.0 / (1.0 + jnp.exp(-cvec)))
    sc8 = jnp.broadcast_to(sc, (8, D)).astype(BF16)

    cp_wq.wait()
    wT_v[pl.ds(0, D), :] = wq_v[...].astype(F32).T.astype(BF16)
    wv_pad = jnp.concatenate(
        [wv_ref[...].astype(F32), jnp.zeros((D, 128 - DH), F32)], axis=1)
    wT_v[pl.ds(D, DH), :] = wv_pad.T[:DH, :].astype(BF16)

    cp_modA.wait()
    modA = jnp.dot(sc8, wmod_v[:, pl.ds(0, 2 * D)], preferred_element_type=F32)
    sa = modA[0:1, 0:D]
    ca1 = 1.0 + modA[0:1, D:2 * D]

    qscale = (DH ** -0.5) * LOG2E
    for b in range(NB):
        cp_x[b].wait()
        if b == NB - 1:
            cp_modB.start()
            cp_wo.start()
            cp_win.start()
            cp_wout.start()
            cp_wsp.start()
        xb = x_v[pl.ds(b * TB, TB), :].astype(F32)
        hb = (_ln(xb) * ca1 + sa).astype(BF16)
        qv = lax.dot_general(wT_v[...], hb, (((1,), (1,)), ((), ())),
                             preferred_element_type=F32)
        qT_v[:, pl.ds(b * TB, TB)] = (qv[:D] * qscale).astype(BF16)
        vT_v[:, pl.ds(b * TB, TB)] = qv[D:].astype(BF16)
        k_v[pl.ds(b * TB, TB), :] = jnp.dot(
            hb, wk_ref[...], preferred_element_type=F32).astype(BF16)

    cp_modB.wait()
    modB = jnp.dot(sc8, wmod_v[:, pl.ds(2 * D, 4 * D)], preferred_element_type=F32)
    mod_v[...] = modB

    def q_tile(t):
        qb = t // H
        h = t % H
        r0 = pl.multiple_of(h * DH, DH)
        c0 = pl.multiple_of(qb * TQ, TQ)
        return qT_v[pl.ds(r0, DH), pl.ds(c0, TQ)]

    def fin_max(mx):
        return jnp.broadcast_to(jnp.max(mx, axis=0, keepdims=True), (8, TQ))

    def pass1_only(t, s_w):
        qt = q_tile(t)
        mx = None
        for c in range(NC):
            s = jnp.dot(k_v[pl.ds(c * TK, TK), :], qt, preferred_element_type=F32)
            s_w[pl.ds(c * TK, TK), :] = s
            cm = jnp.max(s.reshape(TK // 8, 8, TQ), axis=0)
            mx = cm if mx is None else jnp.maximum(mx, cm)
        return fin_max(mx)

    def fused(t, m_cur, s_r, s_w, t_next):
        qt = q_tile(t_next)
        mx = None
        ls = None
        acc = None
        for c in range(NC):
            s = jnp.dot(k_v[pl.ds(c * TK, TK), :], qt, preferred_element_type=F32)
            s_w[pl.ds(c * TK, TK), :] = s
            cm = jnp.max(s.reshape(TK // 8, 8, TQ), axis=0)
            mx = cm if mx is None else jnp.maximum(mx, cm)

            s2 = s_r[pl.ds(c * TK, TK), :].reshape(TK // 8, 8, TQ)
            p = jnp.exp2(s2 - m_cur[None])
            cs = jnp.sum(p, axis=0)
            ls = cs if ls is None else ls + cs
            pb = p.reshape(TK, TQ).astype(BF16)
            pv = jnp.dot(vT_v[:, pl.ds(c * TK, TK)], pb, preferred_element_type=F32)
            acc = pv if acc is None else acc + pv
        l = jnp.sum(ls, axis=0, keepdims=True)
        o = acc * (1.0 / l)
        h = t % H
        r0 = pl.multiple_of(h * DH, DH)
        oT_v[pl.ds(r0, DH), :] = o.astype(BF16)
        return fin_max(mx)

    def block_epilogue(qb):
        r0 = pl.multiple_of(qb * TQ, TQ)
        ga = mod_v[0:1, 0:D]
        sb = mod_v[0:1, D:2 * D]
        cb1 = 1.0 + mod_v[0:1, 2 * D:3 * D]
        y = lax.dot_general(oT_v[...], wo_v[...], (((0,), (0,)), ((), ())),
                            preferred_element_type=F32)
        x1 = x_v[pl.ds(r0, TQ), :].astype(F32) + ga * y
        x1_v[pl.ds(r0, TQ), :] = x1
        h2 = (_ln(x1) * cb1 + sb).astype(BF16)
        z1 = _gelu_tanh(jnp.dot(h2, win_v[:, pl.ds(0, FH)], preferred_element_type=F32))
        z1_v[pl.ds(r0, TQ), :] = z1
        z2 = _gelu_tanh(jnp.dot(h2, win_v[:, pl.ds(FH, FH)], preferred_element_type=F32))
        z2_v[pl.ds(r0, TQ), :] = _ln(z2).astype(BF16)

    NT = NQ * H
    m0 = pass1_only(0, sA_v)
    cp_wo.wait()
    cp_win.wait()

    def pair_body(i, m_a):
        t = 2 * i
        m_b = fused(t, m_a, sA_v, sB_v, t + 1)
        m_a2 = fused(t + 1, m_b, sB_v, sA_v, jnp.minimum(t + 2, NT - 1))

        @pl.when((t + 2) % H == 0)
        def _():
            block_epilogue(t // H)

        return m_a2

    lax.fori_loop(0, NT // 2, pair_body, m0)

    cp_wout.wait()
    cp_wsp.wait()
    gb = mod_v[0:1, 3 * D:4 * D]

    def out_cp(r):
        return pltpu.make_async_copy(out_v.at[r], out_hbm.at[pl.ds(r * TR, TR), :],
                                     osems.at[r])

    for r in range(NR):
        g = jnp.dot(wsp_v[pl.ds(r * TR, TR), :], z2_v[...], preferred_element_type=F32)
        brow = bsp_ref[:, pl.ds(r * TR, TR)].astype(F32)
        bcol = jnp.broadcast_to(brow, (128, TR)).T
        bfull = jnp.concatenate([bcol] * (FH // 128), axis=1)
        u = (z1_v[pl.ds(r * TR, TR), :] * (g + bfull)).astype(BF16)
        yb = jnp.dot(u, wout_v[...], preferred_element_type=F32)
        out_v[r] = (x1_v[pl.ds(r * TR, TR), :] + gb * yb).astype(out_v.dtype)
        out_cp(r).start()
    for r in range(NR):
        out_cp(r).wait()


def make(TQ=512, TK=128, TB=512, TR=512):
    @jax.jit
    def fn(A_x, A_wq, A_wk, A_wv, A_wo, B_x, B_w_in, B_w_sp, B_b_sp, B_w_out, c, w_mod):
        B, S, D = A_x.shape
        DH = A_wk.shape[1]
        H = A_wq.shape[1] // DH
        FH = B_w_in.shape[1] // 2
        NB = S // TB
        NR = S // TR
        x2 = A_x.reshape(S, D)
        bsp = B_b_sp.reshape(1, S)
        any_spec = pl.BlockSpec(memory_space=pl.ANY)
        vm = pl.BlockSpec(memory_space=pltpu.VMEM)
        kern = functools.partial(_kernel, S=S, D=D, H=H, DH=DH, FH=FH,
                                 TQ=TQ, TK=TK, TB=TB, TR=TR)
        out = pl.pallas_call(
            kern,
            out_shape=jax.ShapeDtypeStruct((S, D), A_x.dtype),
            in_specs=[any_spec, any_spec, vm, vm, any_spec, any_spec, any_spec, vm,
                      any_spec, vm, any_spec],
            out_specs=any_spec,
            scratch_shapes=[
                pltpu.VMEM((S, D), BF16),
                pltpu.VMEM((D, D), BF16),
                pltpu.VMEM((D, D), BF16),
                pltpu.VMEM((D, 2 * FH), BF16),
                pltpu.VMEM((S, S), BF16),
                pltpu.VMEM((FH, D), BF16),
                pltpu.VMEM((D, 6 * D), BF16),
                pltpu.VMEM((D + DH, D), BF16),
                pltpu.VMEM((D, S), BF16),
                pltpu.VMEM((S, DH), BF16),
                pltpu.VMEM((DH, S), BF16),
                pltpu.VMEM((S, TQ), F32),
                pltpu.VMEM((S, TQ), F32),
                pltpu.VMEM((D, TQ), BF16),
                pltpu.VMEM((S, D), F32),
                pltpu.VMEM((S, FH), F32),
                pltpu.VMEM((S, FH), BF16),
                pltpu.VMEM((8, 4 * D), F32),
                pltpu.VMEM((NR, TR, D), A_x.dtype),
                pltpu.SemaphoreType.DMA((2 + NB + 5,)),
                pltpu.SemaphoreType.DMA((NR,)),
            ],
            compiler_params=pltpu.CompilerParams(vmem_limit_bytes=100 * 1024 * 1024),
            name="fused_block",
        )(x2, A_wq, A_wk, A_wv, A_wo, B_w_in, B_w_sp, bsp, B_w_out, c, w_mod)
        return out.reshape(B, S, D)
    return fn


_FN = make()


@jax.jit
def pallas_adaLN_cond__grouped_kv_mqa__mixer_gmlp__prompt_kernel(
    A_x: jax.Array,
    A_wq: jax.Array,
    A_wk: jax.Array,
    A_wv: jax.Array,
    A_wo: jax.Array,
    B_x: jax.Array,
    B_w_in: jax.Array,
    B_w_sp: jax.Array,
    B_b_sp: jax.Array,
    B_w_out: jax.Array,
    c: jax.Array,
    w_mod: jax.Array,
):
    return _FN(A_x, A_wq, A_wk, A_wv, A_wo, B_x, B_w_in, B_w_sp, B_b_sp, B_w_out, c, w_mod)
```

```python
import functools
import math

import jax
import jax.numpy as jnp
from jax import lax
import jax.experimental.pallas as pl
import jax.experimental.pallas.tpu as pltpu

F32 = jnp.float32
BF16 = jnp.bfloat16
EPS = 1e-5
LOG2E = 1.4426950408889634


def _ln(x):
    m = jnp.mean(x, axis=-1, keepdims=True)
    xc = x - m
    v = jnp.mean(xc * xc, axis=-1, keepdims=True)
    return xc * lax.rsqrt(v + EPS)


def _gelu_tanh(x):
    c0 = math.sqrt(2.0 / math.pi)
    inner = x * (c0 + (c0 * 0.044715) * (x * x))
    hx = 0.5 * x
    return hx + hx * jnp.tanh(inner)


def _kernel(x_hbm, wq_hbm, wkT_ref, wvT_ref, wo_hbm, win_hbm, wsp_hbm, bsp_ref,
            wout_hbm, c_ref, wmod_hbm, out_hbm,
            x_v, wq_v, wo_v, win_v, wsp_v, wout_v, wmod_v,
            wT_v, h_v, qT_v, k_v, vT_v, sA_v, sB_v, mA_v, mB_v, oT_v, x1_v, z1_v, z2_v,
            mod_v, out_v, sems, osems,
            *, S, D, H, DH, FH, TQ, TK, TB, TE, TR):
    NQ = S // TQ
    NC = S // TK
    NB = S // TB
    NE = S // TE
    NR = S // TR

    def cp(src, dst, i):
        return pltpu.make_async_copy(src, dst, sems.at[i])

    cp_modA = cp(wmod_hbm.at[:, pl.ds(0, 2 * D)], wmod_v.at[:, pl.ds(0, 2 * D)], 0)
    cp_wq = cp(wq_hbm, wq_v, 1)
    cp_x = [cp(x_hbm.at[pl.ds(b * TB, TB), :], x_v.at[pl.ds(b * TB, TB), :], 2 + b)
            for b in range(NB)]
    base = 2 + NB
    cp_modB = cp(wmod_hbm.at[:, pl.ds(2 * D, 4 * D)], wmod_v.at[:, pl.ds(2 * D, 4 * D)], base)
    cp_wo = cp(wo_hbm, wo_v, base + 1)
    cp_win = cp(win_hbm, win_v, base + 2)
    cp_wout = cp(wout_hbm, wout_v, base + 3)
    cp_wsp = cp(wsp_hbm, wsp_v, base + 4)

    cp_modA.start()
    cp_x[0].start()
    cp_wq.start()
    for b in range(1, NB):
        cp_x[b].start()

    cvec = c_ref[...].astype(F32)
    sc = cvec * (1.0 / (1.0 + jnp.exp(-cvec)))
    sc8 = jnp.broadcast_to(sc, (8, D)).astype(BF16)

    cp_modA.wait()
    modA = jnp.dot(sc8, wmod_v[:, pl.ds(0, 2 * D)], preferred_element_type=F32)
    sa = modA[0:1, 0:D]
    ca1 = 1.0 + modA[0:1, D:2 * D]

    qscale = (DH ** -0.5) * LOG2E

    def ln1(b):
        xb = x_v[pl.ds(b * TB, TB), :].astype(F32)
        h_v[pl.ds(b * TB, TB), :] = (_ln(xb) * ca1 + sa).astype(BF16)

    def qkv(b):
        hb = h_v[pl.ds(b * TB, TB), :]
        qv = lax.dot_general(wT_v[...], hb, (((1,), (1,)), ((), ())),
                             preferred_element_type=F32)
        qT_v[:, pl.ds(b * TB, TB)] = (qv[:D] * qscale).astype(BF16)
        vT_v[:, pl.ds(b * TB, TB)] = qv[D:D + DH].astype(BF16)
        k_v[pl.ds(b * TB, TB), :] = qv[D + DH:].T.astype(BF16)

    cp_x[0].wait()
    cp_wq.wait()
    wT_v[pl.ds(0, D), :] = wq_v[...].astype(F32).T.astype(BF16)
    wT_v[pl.ds(D, DH), :] = wvT_ref[...]
    wT_v[pl.ds(D + DH, DH), :] = wkT_ref[...]
    ln1(0)
    for b in range(1, NB):
        cp_x[b].wait()
        if b == NB - 1:
            cp_modB.start()
            cp_wo.start()
            cp_win.start()
            cp_wout.start()
            cp_wsp.start()
        qkv(b - 1)
        ln1(b)
    qkv(NB - 1)

    def q_tile(h, j):
        r0 = pl.multiple_of(h * DH, DH)
        return qT_v[pl.ds(r0, DH), pl.ds(j * TQ, TQ)]

    def fin_max(mx):
        return jnp.broadcast_to(jnp.max(mx, axis=0, keepdims=True), (8, TQ))

    def pass1_only(h, s_w, m_w):
        for j in range(NQ):
            qt = q_tile(h, j)
            mx = None
            for c in range(NC):
                s = jnp.dot(k_v[pl.ds(c * TK, TK), :], qt, preferred_element_type=F32)
                s_w[j, pl.ds(c * TK, TK), :] = s
                cm = jnp.max(s.reshape(TK // 8, 8, TQ), axis=0)
                mx = cm if mx is None else jnp.maximum(mx, cm)
            m_w[j] = fin_max(mx)

    def fused(h, s_r, m_r, s_w, m_w, h_next):
        r0 = pl.multiple_of(h * DH, DH)
        for j in range(NQ):
            qt = q_tile(h_next, j)
            m_cur = m_r[j]
            mx = None
            ls = None
            acc = None
            for c in range(NC):
                s = jnp.dot(k_v[pl.ds(c * TK, TK), :], qt, preferred_element_type=F32)
                s_w[j, pl.ds(c * TK, TK), :] = s
                cm = jnp.max(s.reshape(TK // 8, 8, TQ), axis=0)
                mx = cm if mx is None else jnp.maximum(mx, cm)

                s2 = s_r[j, pl.ds(c * TK, TK), :].reshape(TK // 8, 8, TQ)
                p = jnp.exp2(s2 - m_cur[None])
                cs = jnp.sum(p, axis=0)
                ls = cs if ls is None else ls + cs
                pb = p.reshape(TK, TQ).astype(BF16)
                pv = jnp.dot(vT_v[:, pl.ds(c * TK, TK)], pb, preferred_element_type=F32)
                acc = pv if acc is None else acc + pv
            l = jnp.sum(ls, axis=0, keepdims=True)
            o = acc * (1.0 / l)
            oT_v[pl.ds(r0, DH), pl.ds(j * TQ, TQ)] = o.astype(BF16)
            m_w[j] = fin_max(mx)

    pass1_only(0, sA_v, mA_v)

    def body(h, carry):
        hn = jnp.minimum(h + 1, H - 1)

        @pl.when(h % 2 == 0)
        def _():
            fused(h, sA_v, mA_v, sB_v, mB_v, hn)

        @pl.when(h % 2 == 1)
        def _():
            fused(h, sB_v, mB_v, sA_v, mA_v, hn)

        return carry

    lax.fori_loop(0, H, body, 0)

    cp_modB.wait()
    cp_wo.wait()
    cp_win.wait()
    modB = jnp.dot(sc8, wmod_v[:, pl.ds(2 * D, 4 * D)], preferred_element_type=F32)
    ga = modB[0:1, 0:D]
    sb = modB[0:1, D:2 * D]
    cb1 = 1.0 + modB[0:1, 2 * D:3 * D]
    gb = modB[0:1, 3 * D:4 * D]

    for e in range(NE):
        rows = pl.ds(e * TE, TE)
        y = lax.dot_general(oT_v[:, rows], wo_v[...], (((0,), (0,)), ((), ())),
                            preferred_element_type=F32)
        x1 = x_v[rows, :].astype(F32) + ga * y
        x1_v[rows, :] = x1
        h2 = (_ln(x1) * cb1 + sb).astype(BF16)
        z1 = _gelu_tanh(jnp.dot(h2, win_v[:, pl.ds(0, FH)], preferred_element_type=F32))
        z1_v[rows, :] = z1
        z2 = _gelu_tanh(jnp.dot(h2, win_v[:, pl.ds(FH, FH)], preferred_element_type=F32))
        z2_v[rows, :] = _ln(z2).astype(BF16)

    cp_wout.wait()
    cp_wsp.wait()

    def out_cp(r):
        return pltpu.make_async_copy(out_v.at[r], out_hbm.at[pl.ds(r * TR, TR), :],
                                     osems.at[r])

    for r in range(NR):
        g = jnp.dot(wsp_v[pl.ds(r * TR, TR), :], z2_v[...], preferred_element_type=F32)
        bcols = []
        for i in range(TR // 128):
            brow = bsp_ref[pl.ds(r * (TR // 128) + i, 1), :].astype(F32)
            bcols.append(jnp.broadcast_to(brow, (128, 128)).T)
        bcol = jnp.concatenate(bcols, axis=0)
        bfull = jnp.concatenate([bcol] * (FH // 128), axis=1)
        u = (z1_v[pl.ds(r * TR, TR), :] * (g + bfull)).astype(BF16)
        yb = jnp.dot(u, wout_v[...], preferred_element_type=F32)
        out_v[r] = (x1_v[pl.ds(r * TR, TR), :] + gb * yb).astype(out_v.dtype)
        out_cp(r).start()
    for r in range(NR):
        out_cp(r).wait()


def make(TQ=512, TK=128, TB=512, TE=512, TR=512):
    @jax.jit
    def fn(A_x, A_wq, A_wk, A_wv, A_wo, B_x, B_w_in, B_w_sp, B_b_sp, B_w_out, c, w_mod):
        B, S, D = A_x.shape
        DH = A_wk.shape[1]
        H = A_wq.shape[1] // DH
        FH = B_w_in.shape[1] // 2
        NB = S // TB
        NR = S // TR
        NQ = S // TQ
        x2 = A_x.reshape(S, D)
        bsp = B_b_sp.reshape(S // 128, 128)
        any_spec = pl.BlockSpec(memory_space=pl.ANY)
        vm = pl.BlockSpec(memory_space=pltpu.VMEM)
        kern = functools.partial(_kernel, S=S, D=D, H=H, DH=DH, FH=FH,
                                 TQ=TQ, TK=TK, TB=TB, TE=TE, TR=TR)
        out = pl.pallas_call(
            kern,
            out_shape=jax.ShapeDtypeStruct((S, D), A_x.dtype),
            in_specs=[any_spec, any_spec, vm, vm, any_spec, any_spec, any_spec, vm,
                      any_spec, vm, any_spec],
            out_specs=any_spec,
            scratch_shapes=[
                pltpu.VMEM((S, D), BF16),
                pltpu.VMEM((D, D), BF16),
                pltpu.VMEM((D, D), BF16),
                pltpu.VMEM((D, 2 * FH), BF16),
                pltpu.VMEM((S, S), BF16),
                pltpu.VMEM((FH, D), BF16),
                pltpu.VMEM((D, 6 * D), BF16),
                pltpu.VMEM((D + 2 * DH, D), BF16),
                pltpu.VMEM((S, D), BF16),
                pltpu.VMEM((D, S), BF16),
                pltpu.VMEM((S, DH), BF16),
                pltpu.VMEM((DH, S), BF16),
                pltpu.VMEM((NQ, S, TQ), F32),
                pltpu.VMEM((NQ, S, TQ), F32),
                pltpu.VMEM((NQ, 8, TQ), F32),
                pltpu.VMEM((NQ, 8, TQ), F32),
                pltpu.VMEM((D, S), BF16),
                pltpu.VMEM((S, D), F32),
                pltpu.VMEM((S, FH), F32),
                pltpu.VMEM((S, FH), BF16),
                pltpu.VMEM((8, 4 * D), F32),
                pltpu.VMEM((NR, TR, D), A_x.dtype),
                pltpu.SemaphoreType.DMA((2 + NB + 5,)),
                pltpu.SemaphoreType.DMA((NR,)),
            ],
            compiler_params=pltpu.CompilerParams(vmem_limit_bytes=110 * 1024 * 1024),
            name="fused_block",
        )(x2, A_wq, A_wk.T, A_wv.T, A_wo, B_w_in, B_w_sp, bsp, B_w_out, c, w_mod)
        return out.reshape(B, S, D)
    return fn


_FN = make()


@jax.jit
def pallas_adaLN_cond__grouped_kv_mqa__mixer_gmlp__prompt_kernel(
    A_x: jax.Array,
    A_wq: jax.Array,
    A_wk: jax.Array,
    A_wv: jax.Array,
    A_wo: jax.Array,
    B_x: jax.Array,
    B_w_in: jax.Array,
    B_w_sp: jax.Array,
    B_b_sp: jax.Array,
    B_w_out: jax.Array,
    c: jax.Array,
    w_mod: jax.Array,
):
    return _FN(A_x, A_wq, A_wk, A_wv, A_wo, B_x, B_w_in, B_w_sp, B_b_sp, B_w_out, c, w_mod)
```

```python
import functools
import math

import jax
import jax.numpy as jnp
from jax import lax
import jax.experimental.pallas as pl
import jax.experimental.pallas.tpu as pltpu

F32 = jnp.float32
BF16 = jnp.bfloat16
U32 = jnp.uint32
EPS = 1e-5
LOG2E = 1.4426950408889634
L_MIN = 2.0 ** -60


def _ln(x):
    m = jnp.mean(x, axis=-1, keepdims=True)
    xc = x - m
    v = jnp.mean(xc * xc, axis=-1, keepdims=True)
    return xc * lax.rsqrt(v + EPS)


def _gelu_tanh(x):
    c0 = math.sqrt(2.0 / math.pi)
    inner = x * (c0 + (c0 * 0.044715) * (x * x))
    hx = 0.5 * x
    return hx + hx * jnp.tanh(inner)


def _b(x):
    return pltpu.bitcast(x, BF16)


def _u(x):
    return pltpu.bitcast(x, U32)


def _kernel(x_hbm, wq_hbm, wkT_ref, wvT_ref, wo_hbm, win_hbm, wsp_hbm, bsp_ref,
            wout_hbm, c_ref, wmod_hbm, out_hbm,
            x_v, wq_v, wo_v, win_v, wsp_v, wout_v, wmod_v,
            wT_v, h_v, qa_v, q32_v, nm_v, ka_v, kb_v, vT_v,
            pA_v, pB_v, lA_v, lB_v, sA_v, sB_v, bad_v, oT_v, x1_v, z1_v, z2_v,
            out_v, sems, osems,
            *, S, D, H, DH, FH, TQ, TK, TB, TE, TR, NV, G, SL):
    NQ = S // TQ
    NC = S // TK
    NB = S // TB
    NE = S // TE
    NR = S // TR
    NT = TQ // 128

    def cp(src, dst, i):
        return pltpu.make_async_copy(src, dst, sems.at[i])

    cp_modA = cp(wmod_hbm.at[:, pl.ds(0, 2 * D)], wmod_v.at[:, pl.ds(0, 2 * D)], 0)
    cp_wq = cp(wq_hbm, wq_v, 1)
    cp_x = [cp(x_hbm.at[pl.ds(b * TB, TB), :], x_v.at[pl.ds(b * TB, TB), :], 2 + b)
            for b in range(NB)]
    base = 2 + NB
    cp_modB = cp(wmod_hbm.at[:, pl.ds(2 * D, 4 * D)], wmod_v.at[:, pl.ds(2 * D, 4 * D)], base)
    cp_wo = cp(wo_hbm, wo_v, base + 1)
    cp_win = cp(win_hbm, win_v, base + 2)
    cp_wout = cp(wout_hbm, wout_v, base + 3)
    cp_wsp = cp(wsp_hbm, wsp_v, base + 4)

    cp_modA.start()
    cp_x[0].start()
    cp_wq.start()
    for b in range(1, NB):
        cp_x[b].start()

    cvec = c_ref[...].astype(F32)
    sc = cvec * (1.0 / (1.0 + jnp.exp(-cvec)))
    sc8 = jnp.broadcast_to(sc, (8, D)).astype(BF16)
    bad_v[...] = jnp.zeros(bad_v.shape, F32)

    e_r = lax.broadcasted_iota(jnp.int32, (H, D), 0)
    e_c = lax.broadcasted_iota(jnp.int32, (H, D), 1)
    emat = jnp.where((e_c >= e_r * DH) & (e_c < (e_r + 1) * DH), 1.0, 0.0).astype(BF16)
    aug_r = lax.broadcasted_iota(jnp.int32, (DH, TB), 0)
    aug = jnp.where(aug_r < 2, 1.0, 0.0).astype(F32)

    cp_modA.wait()
    modA = jnp.dot(sc8, wmod_v[:, pl.ds(0, 2 * D)], preferred_element_type=F32)
    sa = modA[0:1, 0:D]
    ca1 = 1.0 + modA[0:1, D:2 * D]

    qscale = (DH ** -0.5) * LOG2E

    def ln1(b):
        xb = x_v[pl.ds(b * TB, TB), :].astype(F32)
        h_v[pl.ds(b * TB, TB), :] = (_ln(xb) * ca1 + sa).astype(BF16)

    kst = {}

    def qkv(b):
        cols = pl.ds(b * TB, TB)
        hb = h_v[cols, :]
        qv = lax.dot_general(wT_v[...], hb, (((1,), (1,)), ((), ())),
                             preferred_element_type=F32)
        qs = qv[:D] * qscale
        qa_v[:, cols] = _u(qs.astype(BF16))
        q32_v[:, :, cols] = qs.reshape(H, DH, TB)
        qn2 = jnp.dot(emat, (qs * qs).astype(BF16), preferred_element_type=F32)
        for t in range(TB // 128):
            nm_v[b * (TB // 128) + t] = qn2[:, t * 128:(t + 1) * 128]
        vT_v[:, cols] = _u(qv[D:D + DH].astype(BF16))
        kT = qv[D + DH:]
        k2 = jnp.sum(kT * kT, axis=0, keepdims=True)
        kst['k2'] = k2 if b == 0 else jnp.maximum(kst['k2'], k2)
        kaug = jnp.concatenate([kT, aug], axis=0).T
        ka_v[pl.ds(b * TB // 2, TB // 2), :] = _u(kaug.astype(BF16))
        if b == 0:
            for d in range(DH):
                kb_v[d] = jnp.broadcast_to(kaug[:NV, d:d + 1], (NV, 128))

    cp_x[0].wait()
    cp_wq.wait()
    wT_v[pl.ds(0, D), :] = wq_v[...].astype(F32).T.astype(BF16)
    wT_v[pl.ds(D, DH), :] = wvT_ref[...]
    wT_v[pl.ds(D + DH, DH), :] = wkT_ref[...]
    ln1(0)
    for b in range(1, NB):
        cp_x[b].wait()
        if b == NB - 1:
            cp_modB.start()
            cp_wo.start()
            cp_win.start()
            cp_wout.start()
            cp_wsp.start()
        qkv(b - 1)
        ln1(b)
    qkv(NB - 1)

    kmax = jnp.sqrt(jnp.max(kst['k2'], axis=1, keepdims=True)) * (-1.015625)
    for t in range(S // 128):
        nm_v[t] = (jnp.sqrt(nm_v[t]) * kmax).astype(BF16).astype(F32)

    def nm_row(h, c0):
        return nm_v[c0 // 128, pl.ds(h, 1), :]

    def q_tile(h, j):
        r0 = pl.multiple_of(h * (DH // 2), DH // 2)
        q = qa_v[pl.ds(r0, DH // 2), pl.ds(j * TQ, TQ)]
        m = jnp.concatenate(
            [jnp.broadcast_to(nm_row(h, j * TQ + t * 128), (DH // 2, 128)) for t in range(NT)],
            axis=1)
        return _b(jnp.concatenate([q, pltpu.bitcast(m, U32)], axis=0))

    class Piece:
        def __init__(s, h, j, g, w):
            s.h, s.j, s.g, s.w = h, j, g, w
            s.a = None
            s.d = 0

        def step(s):
            c0 = [s.j * TQ + t * 128 for t in range(NT)]
            if s.a is None:
                s.a = [jnp.broadcast_to(nm_row(s.h, c0[t]), (G, 128)) for t in range(NT)]
            kb = kb_v[s.d, pl.ds(s.g * G, G), :]
            for t in range(NT):
                s.a[t] = s.a[t] + kb * q32_v[s.h, pl.ds(s.d, 1), pl.ds(c0[t], 128)]
            s.d += 1

        def fin(s):
            s.w[s.j, pl.ds(s.g * G, G), :] = jnp.concatenate(s.a, axis=1)

    def pv_chunk(p_r, j, cc):
        pb = _b(p_r[pl.ds(cc * TK // 2, TK // 2), pl.ds(j * TQ, TQ)])
        return jnp.dot(_b(vT_v[:, pl.ds(cc * TK, TK)]), pb, preferred_element_type=F32)

    def pv_fin(hp, j, acc, l_r, check=True):
        cols = pl.ds(j * TQ, TQ)
        l = jnp.sum(l_r[j], axis=0, keepdims=True)
        r0 = pl.multiple_of(hp * (DH // 2), DH // 2)
        oT_v[pl.ds(r0, DH // 2), cols] = _u((acc * (1.0 / l)).astype(BF16))
        if check:
            bad_v[:, cols] = jnp.where(l >= L_MIN, bad_v[:, cols], 1.0)

    def it(h, p_r, l_r, p_w, l_w, s_r, s_w):
        first = s_r is None
        hf = jnp.minimum(h + 1, H - 1)
        k0 = 0 if first else NV
        for j in range(NQ):
            stream = []
            for g in range(NV // G):
                pc = Piece(hf, j, g, s_w)
                stream += [pc.step] * DH + [pc.fin]
            total_slabs = (S - k0) // SL
            st = dict(i=0, slab=0, l=None)

            def emit_fma():
                st['slab'] += 1
                tgt = min(len(stream), -(-st['slab'] * len(stream) // total_slabs))
                while st['i'] < tgt:
                    stream[st['i']]()
                    st['i'] += 1

            def slabs(s, row0, n, emit):
                for r in range(n // SL):
                    p = jnp.exp2(s[r * SL:(r + 1) * SL])
                    cs = jnp.sum(p.reshape(SL // 8, 8, TQ), axis=0)
                    st['l'] = cs if st['l'] is None else st['l'] + cs
                    p_w[pl.ds((row0 + r * SL) // 2, SL // 2), pl.ds(j * TQ, TQ)] = _u(p.astype(BF16))
                    if emit:
                        emit_fma()

            acc = None
            nqc = -(-(S - k0) // TK)
            rawrows = [] if first else list(range(0, NV, SL))
            nr = len(rawrows)
            pvs = [] if first else list(range(NC))
            for c in range(nqc):
                lo = k0 + c * TK
                hi = min(lo + TK, S)
                s = jnp.dot(_b(ka_v[pl.ds(lo // 2, (hi - lo) // 2), :]), q_tile(h, j),
                            preferred_element_type=F32)
                slabs(s, lo, hi - lo, True)
                while len(rawrows) > nr - -(-(c + 1) * nr // nqc):
                    r0 = rawrows.pop(0)
                    slabs(s_r[j, pl.ds(r0, SL), :], r0, SL, False)
                while len(pvs) > NC - -(-(c + 1) * NC // nqc):
                    pv = pv_chunk(p_r, j, pvs.pop(0))
                    acc = pv if acc is None else acc + pv
            while st['i'] < len(stream):
                stream[st['i']]()
                st['i'] += 1
            l_w[j] = st['l']
            if not first:
                pv_fin(h - 1, j, acc, l_r)

    it(0, None, None, pA_v, lA_v, None, sB_v)

    def body(h, carry):
        @pl.when(h % 2 == 1)
        def _():
            it(h, pA_v, lA_v, pB_v, lB_v, sB_v, sA_v)

        @pl.when(h % 2 == 0)
        def _():
            it(h, pB_v, lB_v, pA_v, lA_v, sA_v, sB_v)

        return carry

    lax.fori_loop(1, H, body, 0)

    pL_v, lL_v = (pB_v, lB_v) if (H - 1) % 2 == 1 else (pA_v, lA_v)
    badf = bad_v[...]
    lastl = jnp.concatenate([jnp.sum(lL_v[j], axis=0, keepdims=True) for j in range(NQ)], axis=1)
    badf = jnp.where(lastl >= L_MIN, badf, 1.0)

    @pl.when(jnp.max(badf) > 0.5)
    def _():
        def fb(h, carry):
            r0 = pl.multiple_of(h * (DH // 2), DH // 2)
            for j in range(NQ):
                cols = pl.ds(j * TQ, TQ)
                qt = _b(jnp.concatenate([qa_v[pl.ds(r0, DH // 2), cols],
                                         jnp.zeros((DH // 2, TQ), U32)], axis=0))

                def sc_(c):
                    k0 = pl.multiple_of(c * (TK // 2), TK // 2)
                    return jnp.dot(_b(ka_v[pl.ds(k0, TK // 2), :]), qt,
                                   preferred_element_type=F32)

                def p1(c, mx):
                    return jnp.maximum(mx, jnp.max(sc_(c).reshape(TK // 8, 8, TQ), axis=0))

                mx = lax.fori_loop(0, NC, p1, jnp.full((8, TQ), -jnp.inf, F32))
                m = jnp.max(mx, axis=0, keepdims=True)

                def p2(c, ls):
                    p = jnp.exp2(sc_(c) - m)
                    k0 = pl.multiple_of(c * (TK // 2), TK // 2)
                    pL_v[pl.ds(k0, TK // 2), cols] = _u(p.astype(BF16))
                    return ls + jnp.sum(p.reshape(TK // 8, 8, TQ), axis=0)

                lL_v[j] = lax.fori_loop(0, NC, p2, jnp.zeros((8, TQ), F32))
                acc = jnp.dot(_b(vT_v[...]), _b(pL_v[:, cols]), preferred_element_type=F32)
                pv_fin(h, j, acc, lL_v, check=False)
            return carry

        lax.fori_loop(0, H, fb, 0)

    cp_modB.wait()
    cp_wo.wait()
    cp_win.wait()
    modB = jnp.dot(sc8, wmod_v[:, pl.ds(2 * D, 4 * D)], preferred_element_type=F32)
    ga = modB[0:1, 0:D]
    sb = modB[0:1, D:2 * D]
    cb1 = 1.0 + modB[0:1, 2 * D:3 * D]
    gb = modB[0:1, 3 * D:4 * D]

    for j in range(NQ):
        acc = None
        for cc in range(NC):
            pv = pv_chunk(pL_v, j, cc)
            acc = pv if acc is None else acc + pv
        pv_fin(H - 1, j, acc, lL_v, check=False)

    for e in range(NE):
        rows = pl.ds(e * TE, TE)
        y = lax.dot_general(_b(oT_v[:, rows]), wo_v[...], (((0,), (0,)), ((), ())),
                            preferred_element_type=F32)
        x1 = x_v[rows, :].astype(F32) + ga * y
        x1_v[rows, :] = x1
        h2 = (_ln(x1) * cb1 + sb).astype(BF16)
        z1 = _gelu_tanh(jnp.dot(h2, win_v[:, pl.ds(0, FH)], preferred_element_type=F32))
        z1_v[rows, :] = z1
        z2 = _gelu_tanh(jnp.dot(h2, win_v[:, pl.ds(FH, FH)], preferred_element_type=F32))
        z2_v[rows, :] = _ln(z2).astype(BF16)

    cp_wout.wait()
    cp_wsp.wait()

    def out_cp(r):
        return pltpu.make_async_copy(out_v.at[r], out_hbm.at[pl.ds(r * TR, TR), :],
                                     osems.at[r])

    for r in range(NR):
        g = jnp.dot(wsp_v[pl.ds(r * TR, TR), :], z2_v[...], preferred_element_type=F32)
        bcols = []
        for i in range(TR // 128):
            brow = bsp_ref[pl.ds(r * (TR // 128) + i, 1), :].astype(F32)
            bcols.append(jnp.broadcast_to(brow, (128, 128)).T)
        bcol = jnp.concatenate(bcols, axis=0)
        bfull = jnp.concatenate([bcol] * (FH // 128), axis=1)
        u = (z1_v[pl.ds(r * TR, TR), :] * (g + bfull)).astype(BF16)
        yb = jnp.dot(u, wout_v[...], preferred_element_type=F32)
        out_v[r] = (x1_v[pl.ds(r * TR, TR), :] + gb * yb).astype(out_v.dtype)
        out_cp(r).start()
    for r in range(NR):
        out_cp(r).wait()


def make(TQ=512, TK=128, TB=512, TE=512, TR=512, NV=192, G=16, SL=16):
    @jax.jit
    def fn(A_x, A_wq, A_wk, A_wv, A_wo, B_x, B_w_in, B_w_sp, B_b_sp, B_w_out, c, w_mod):
        B, S, D = A_x.shape
        DH = A_wk.shape[1]
        H = A_wq.shape[1] // DH
        FH = B_w_in.shape[1] // 2
        NB = S // TB
        NR = S // TR
        NQ = S // TQ
        x2 = A_x.reshape(S, D)
        bsp = B_b_sp.reshape(S // 128, 128)
        any_spec = pl.BlockSpec(memory_space=pl.ANY)
        vm = pl.BlockSpec(memory_space=pltpu.VMEM)
        kern = functools.partial(_kernel, S=S, D=D, H=H, DH=DH, FH=FH,
                                 TQ=TQ, TK=TK, TB=TB, TE=TE, TR=TR, NV=NV, G=G, SL=SL)
        out = pl.pallas_call(
            kern,
            out_shape=jax.ShapeDtypeStruct((S, D), A_x.dtype),
            in_specs=[any_spec, any_spec, vm, vm, any_spec, any_spec, any_spec, vm,
                      any_spec, vm, any_spec],
            out_specs=any_spec,
            scratch_shapes=[
                pltpu.VMEM((S, D), BF16),
                pltpu.VMEM((D, D), BF16),
                pltpu.VMEM((D, D), BF16),
                pltpu.VMEM((D, 2 * FH), BF16),
                pltpu.VMEM((S, S), BF16),
                pltpu.VMEM((FH, D), BF16),
                pltpu.VMEM((D, 6 * D), BF16),
                pltpu.VMEM((D + 2 * DH, D), BF16),
                pltpu.VMEM((S, D), BF16),
                pltpu.VMEM((D // 2, S), U32),
                pltpu.VMEM((H, DH, S), F32),
                pltpu.VMEM((S // 128, H, 128), F32),
                pltpu.VMEM((S // 2, 2 * DH), U32),
                pltpu.VMEM((DH, NV, 128), F32),
                pltpu.VMEM((DH // 2, S), U32),
                pltpu.VMEM((S // 2, S), U32),
                pltpu.VMEM((S // 2, S), U32),
                pltpu.VMEM((NQ, 8, TQ), F32),
                pltpu.VMEM((NQ, 8, TQ), F32),
                pltpu.VMEM((NQ, NV, TQ), F32),
                pltpu.VMEM((NQ, NV, TQ), F32),
                pltpu.VMEM((1, S), F32),
                pltpu.VMEM((D // 2, S), U32),
                pltpu.VMEM((S, D), F32),
                pltpu.VMEM((S, FH), F32),
                pltpu.VMEM((S, FH), BF16),
                pltpu.VMEM((NR, TR, D), A_x.dtype),
                pltpu.SemaphoreType.DMA((2 + NB + 5,)),
                pltpu.SemaphoreType.DMA((NR,)),
            ],
            compiler_params=pltpu.CompilerParams(vmem_limit_bytes=110 * 1024 * 1024),
            name="fused_block",
        )(x2, A_wq, A_wk.T, A_wv.T, A_wo, B_w_in, B_w_sp, bsp, B_w_out, c, w_mod)
        return out.reshape(B, S, D)
    return fn


_FN = make()


@jax.jit
def pallas_adaLN_cond__grouped_kv_mqa__mixer_gmlp__prompt_kernel(
    A_x: jax.Array,
    A_wq: jax.Array,
    A_wk: jax.Array,
    A_wv: jax.Array,
    A_wo: jax.Array,
    B_x: jax.Array,
    B_w_in: jax.Array,
    B_w_sp: jax.Array,
    B_b_sp: jax.Array,
    B_w_out: jax.Array,
    c: jax.Array,
    w_mod: jax.Array,
):
    return _FN(A_x, A_wq, A_wk, A_wv, A_wo, B_x, B_w_in, B_w_sp, B_b_sp, B_w_out, c, w_mod)
```

```python
import functools
import math

import jax
import jax.numpy as jnp
from jax import lax
import jax.experimental.pallas as pl
import jax.experimental.pallas.tpu as pltpu

F32 = jnp.float32
BF16 = jnp.bfloat16
U32 = jnp.uint32
EPS = 1e-5
LOG2E = 1.4426950408889634
L_MIN = 2.0 ** -60


def _ln(x):
    m = jnp.mean(x, axis=-1, keepdims=True)
    xc = x - m
    v = jnp.mean(xc * xc, axis=-1, keepdims=True)
    return xc * lax.rsqrt(v + EPS)


def _gelu_tanh(x):
    c0 = math.sqrt(2.0 / math.pi)
    inner = x * (c0 + (c0 * 0.044715) * (x * x))
    hx = 0.5 * x
    return hx + hx * jnp.tanh(inner)


PROF = False


class _Null:
    def __enter__(self):
        return self

    def __exit__(self, *a):
        return False


def _scope(name):
    return jax.named_scope(name) if PROF else _Null()


def _b(x):
    return pltpu.bitcast(x, BF16)


def _u(x):
    return pltpu.bitcast(x, U32)


def _kernel(x_hbm, wq_hbm, wkT_hbm, wvT_hbm, wo_hbm, win_hbm, wsp_hbm, bsp_hbm,
            wout_hbm, c_hbm, wmod_hbm, out_hbm,
            x_v, wq_v, wo_v, win_v, wsp_v, wout_v, wmod_v, wmA_v,
            wT_v, h_v, qa_v, q32_v, nm_v, ka_v, kb_v, vT_v,
            pA_v, pB_v, lA_v, lB_v, sA_v, sB_v, bad_v, oT_v, x1_v, z1_v, z2_v,
            out_v, hu_v, wkT_v, wvT_v, bsp_ref, c_v, sems, osems,
            *, S, D, H, DH, FH, TQ, TK, XB, LL, TE, TR, NV, G, SL, EBAR, OPQ, TCH, KB0, KB1, TKA, TL, TLU, MSPL):
    NQ = S // TQ
    NC = S // TK
    NE = S // TE
    NR = S // TR
    NT = TQ // 128

    def cp(src, dst, i):
        return pltpu.make_async_copy(src, dst, sems.at[i])

    UT = 128
    NU = S // UT
    xb = [0] + list(XB) + [S]
    NX = len(xb) - 1
    NMA = MSPL
    cp_modAs = [cp(wmod_hbm.at[pl.ds(i * D // NMA, D // NMA), pl.ds(0, 2 * D)], wmA_v.at[pl.ds(i * D // NMA, D // NMA), :], 0 if i == 0 else 6 + NX + 5 + i) for i in range(NMA)]
    cp_wq = cp(wq_hbm, wq_v, 1)
    cp_c = cp(c_hbm, c_v, 2)
    cp_wk = cp(wkT_hbm, wkT_v, 3)
    cp_wv = cp(wvT_hbm, wvT_v, 4)
    cp_bsp = cp(bsp_hbm, bsp_ref, 5)
    cp_x = [cp(x_hbm.at[pl.ds(xb[i], xb[i + 1] - xb[i]), :],
               x_v.at[pl.ds(xb[i], xb[i + 1] - xb[i]), :], 6 + i) for i in range(NX)]
    base = 6 + NX
    cp_modB = cp(wmod_hbm.at[:, pl.ds(2 * D, 4 * D)], wmod_v, base)
    cp_wo = cp(wo_hbm, wo_v, base + 1)
    cp_win = cp(win_hbm, win_v, base + 2)
    cp_wout = cp(wout_hbm, wout_v, base + 3)
    cp_wsp = cp(wsp_hbm.at[pl.ds(0, S // 2), :], wsp_v.at[pl.ds(0, S // 2), :], base + 4)
    cp_wo2 = cp(wsp_hbm.at[pl.ds(S // 2, S // 2), :], wsp_v.at[pl.ds(S // 2, S // 2), :], base + 5)

    def wait(c, name):
        with _scope("w_" + name):
            c.wait()

    for c_ in [cp_wq, cp_x[0], cp_c, cp_wk, cp_wv] + cp_modAs + cp_x[1:]:
        c_.start()

    zer = lax.fori_loop(0, 2, lambda i, c: c * i, jnp.int32(1))

    def dd(r0, n):
        return pl.ds(pl.multiple_of(zer * 16 + r0, 8), n) if OPQ else pl.ds(r0, n)

    zer_u = zer.astype(U32)

    def tie(x, vals):
        t = None
        for v in vals:
            w = v if v.dtype == U32 else pltpu.bitcast(v, U32)
            for r in range(w.shape[0] // 8):
                for c in range(w.shape[1] // 128):
                    p = w[r * 8:(r + 1) * 8, c * 128:(c + 1) * 128]
                    t = p if t is None else t | p
        if t is None:
            return x
        top = x[:8, :128] | (t & zer_u)
        if x.shape[1] > 128:
            top = jnp.concatenate([top, x[:8, 128:]], axis=1)
        return jnp.concatenate([top, x[8:]], axis=0)

    bad_v[...] = jnp.zeros(bad_v.shape, F32)
    e_r = lax.broadcasted_iota(jnp.int32, (H, D), 0)
    e_c = lax.broadcasted_iota(jnp.int32, (H, D), 1)
    emat = jnp.where((e_c >= e_r * DH) & (e_c < (e_r + 1) * DH), 1.0, 0.0).astype(BF16)
    aug_r = lax.broadcasted_iota(jnp.int32, (DH, UT), 0)
    aug = jnp.where(aug_r < 2, 1.0, 0.0).astype(F32)
    qscale = (DH ** -0.5) * LOG2E

    wait(cp_wq, 'wq')
    wT_v[pl.ds(0, D // 2), :] = _u(wq_v[...].astype(F32).T.astype(BF16))
    wait(cp_x[0], 'x0')
    x1_v[pl.ds(0, xb[1]), :] = _ln(x_v[pl.ds(0, xb[1]), :].astype(F32))
    wait(cp_c, 'c')
    wait(cp_wk, 'wk')
    wait(cp_wv, 'wv')
    wT_v[pl.ds(D // 2, DH // 2), :] = _u(wvT_v[...])
    wT_v[pl.ds((D + DH) // 2, DH // 2), :] = _u(wkT_v[...])
    cvec = c_v[...].astype(F32)
    sc = cvec * (1.0 / (1.0 + jnp.exp(-cvec)))
    sc8 = jnp.broadcast_to(sc, (8, D)).astype(BF16)

    for c_ in cp_modAs:
        wait(c_, 'modA')
    modA = jnp.dot(sc8, wmA_v[...], preferred_element_type=F32)
    sa = modA[0:1, 0:D]
    ca1 = 1.0 + modA[0:1, D:2 * D]

    def ln1(r0, n):
        if r0 < xb[1]:
            xh = x1_v[dd(r0, n), :]
        else:
            xh = _ln(x_v[pl.ds(r0, n), :].astype(F32))
        hv = _u((xh * ca1 + sa).astype(BF16))
        hu_v[pl.ds(r0 // 2, n // 2), :] = hv
        return hv

    kst = {}
    NT_ = (((1,), (1,)), ((), ()))

    kbd = {}
    for d in range(DH):
        kbd.setdefault(KB0 + d * (KB1 - KB0) // DH, []).append(d)

    def norms(u):
        qn2 = jnp.dot(emat, jnp.concatenate(kst.pop(u), axis=0), preferred_element_type=F32)
        nm_v[u] = jnp.sqrt(qn2)

    def qkv(u):
        sq = kst[u] = []
        cols = pl.ds(u * UT, UT)
        hb = _b(hu_v[dd(u * UT // 2, UT // 2), :])
        un = u + LL
        nch = D // 128
        for ch in range(nch):
            last = ch == nch - 1
            nrow = 128 + (2 * DH if last else 0)
            wch = wT_v[dd(ch * 64, nrow // 2), :]
            tl = kst.pop(('ln', u * nch + ch), [])
            if ch == TCH:
                tl = tl + kst.pop('tie', [])
            wch = tie(wch, tl)
            qv = lax.dot_general(_b(wch), hb, NT_,
                                 preferred_element_type=F32)
            qs = qv[:128] * qscale
            qa_v[pl.ds(ch * 64, 64), cols] = _u(qs.astype(BF16))
            q32_v[pl.ds(ch * 8, 8), :, cols] = qs.reshape(8, DH, UT)
            sq.append((qs * qs).astype(BF16))
            if ch == 1 and u > 0:
                norms(u - 1)
            if last:
                vT_v[:, cols] = _u(qv[128:128 + DH].astype(BF16))
                kT = qv[128 + DH:]
                k2 = jnp.sum(kT * kT, axis=0, keepdims=True)
                kst['k2'] = k2 if u == 0 else jnp.maximum(kst['k2'], k2)
                kaug = jnp.concatenate([kT, aug], axis=0).T
                kau = _u(kaug.astype(BF16))
                ka_v[pl.ds(u * UT // 2, UT // 2), :] = kau
                nkb = min(UT, NV - u * UT)
                if nkb > 0:
                    kst.setdefault('kf', []).append(kaug[:nkb])
                if TKA:
                    kst.setdefault(('ln', (u + 1) * nch + TKA), []).append(
                        jnp.concatenate([kau, jnp.zeros((UT // 2, 128 - 2 * DH), U32)], axis=1))
                tv = []
                for d in kbd.get(u, []):
                    kf = jnp.concatenate(kst['kf'], axis=0)
                    kbv = jnp.broadcast_to(kf[:, d:d + 1], (NV, 128))
                    kb_v[d] = kbv
                    tv.append(kbv)
                kst['tie'] = tv
            if un < NU:
                hv = ln1(un * UT + ch * (UT // nch), UT // nch)
                if TL and un in TLU:
                    kst.setdefault(('ln', u * nch + ch + TL), []).append(hv)

    nx = 1
    for u in range(NU):
        need = min(u + LL + 1, NU) * UT
        while nx < NX and xb[nx] < need:
            wait(cp_x[nx], 'x%d' % nx)
            nx += 1
        if u == 0:
            for v in range(LL):
                ln1(v * UT, UT)
        qkv(u)
    norms(NU - 1)

    kmax = jnp.sqrt(jnp.max(kst['k2'], axis=1, keepdims=True)) * (-1.015625)
    for t in range(S // 128):
        nm_v[t] = (nm_v[t] * kmax).astype(BF16).astype(F32)

    def nm_row(h, c0):
        return nm_v[c0 // 128, pl.ds(h, 1), :]

    def q_tile(h, j):
        r0 = pl.multiple_of(h * (DH // 2), DH // 2)
        q = qa_v[pl.ds(r0, DH // 2), pl.ds(j * TQ, TQ)]
        m = jnp.concatenate(
            [jnp.broadcast_to(nm_row(h, j * TQ + t * 128), (DH // 2, 128)) for t in range(NT)],
            axis=1)
        return _b(jnp.concatenate([q, pltpu.bitcast(m, U32)], axis=0))

    class Piece:
        def __init__(s, h, j, g, w):
            s.h, s.j, s.g, s.w = h, j, g, w
            s.a = None
            s.d = 0

        def step(s):
            c0 = [s.j * TQ + t * 128 for t in range(NT)]
            if s.a is None:
                s.a = [jnp.broadcast_to(nm_row(s.h, c0[t]), (G, 128)) for t in range(NT)]
            kb = kb_v[s.d, pl.ds(s.g * G, G), :]
            for t in range(NT):
                s.a[t] = s.a[t] + kb * q32_v[s.h, pl.ds(s.d, 1), pl.ds(c0[t], 128)]
            s.d += 1

        def fin(s):
            s.w[s.j, pl.ds(s.g * G, G), :] = jnp.concatenate(s.a, axis=1)

    def pv_chunk(p_r, j, cc):
        pb = _b(p_r[pl.ds(cc * TK // 2, TK // 2), pl.ds(j * TQ, TQ)])
        return jnp.dot(_b(vT_v[:, pl.ds(cc * TK, TK)]), pb, preferred_element_type=F32)

    def pv_fin(hp, j, acc, l_r, check=True):
        cols = pl.ds(j * TQ, TQ)
        l = jnp.sum(l_r[j], axis=0, keepdims=True)
        r0 = pl.multiple_of(hp * (DH // 2), DH // 2)
        oT_v[pl.ds(r0, DH // 2), cols] = _u((acc * (1.0 / l)).astype(BF16))
        if check:
            bad_v[:, cols] = jnp.where(l >= L_MIN, bad_v[:, cols], 1.0)

    def it(h, p_r, l_r, p_w, l_w, s_r, s_w):
        first = s_r is None
        hf = jnp.minimum(h + 1, H - 1)
        k0 = 0 if first else NV
        for j in range(NQ):
            stream = []
            for g in range(NV // G):
                pc = Piece(hf, j, g, s_w)
                stream += [pc.step] * DH + [pc.fin]
            total_slabs = (S - k0) // SL
            st = dict(i=0, slab=0, l=None)

            def emit_fma():
                st['slab'] += 1
                tgt = min(len(stream), -(-st['slab'] * len(stream) // total_slabs))
                while st['i'] < tgt:
                    stream[st['i']]()
                    st['i'] += 1

            def slabs(s, row0, n, emit):
                for r in range(n // SL):
                    p = jnp.exp2(s[r * SL:(r + 1) * SL])
                    cs = jnp.sum(p.reshape(SL // 8, 8, TQ), axis=0)
                    st['l'] = cs if st['l'] is None else st['l'] + cs
                    p_w[pl.ds((row0 + r * SL) // 2, SL // 2), pl.ds(j * TQ, TQ)] = _u(p.astype(BF16))
                    if emit:
                        emit_fma()

            acc = None
            nqc = -(-(S - k0) // TK)
            rawrows = [] if first else list(range(0, NV, SL))
            nr = len(rawrows)
            pvs = [] if first else list(range(NC))
            for c in range(nqc):
                lo = k0 + c * TK
                hi = min(lo + TK, S)
                s = jnp.dot(_b(ka_v[pl.ds(lo // 2, (hi - lo) // 2), :]), q_tile(h, j),
                            preferred_element_type=F32)
                slabs(s, lo, hi - lo, True)
                while len(rawrows) > nr - -(-(c + 1) * nr // nqc):
                    r0 = rawrows.pop(0)
                    slabs(s_r[j, pl.ds(r0, SL), :], r0, SL, False)
                while len(pvs) > NC - -(-(c + 1) * NC // nqc):
                    pv = pv_chunk(p_r, j, pvs.pop(0))
                    acc = pv if acc is None else acc + pv
            while st['i'] < len(stream):
                stream[st['i']]()
                st['i'] += 1
            l_w[j] = st['l']
            if not first:
                pv_fin(h - 1, j, acc, l_r)

    def pair(i, carry):
        @pl.when(2 * i + 1 < H)
        def _():
            it(2 * i + 1, pA_v, lA_v, pB_v, lB_v, sB_v, sA_v)

        @pl.when(2 * i + 2 < H)
        def _():
            it(2 * i + 2, pB_v, lB_v, pA_v, lA_v, sA_v, sB_v)

        return carry

    def outer(t, carry):
        @pl.when(t == 0)
        def _():
            it(t, None, None, pA_v, lA_v, None, sB_v)

        @pl.when(t == 2)
        def _():
            for c_ in [cp_wo, cp_modB, cp_win, cp_wout, cp_wsp, cp_wo2, cp_bsp]:
                c_.start()

        @pl.when(t >= 1)
        def _():
            lax.fori_loop(t - 1, jnp.where(t == 1, 1, H // 2), pair, 0)

        return carry

    with _scope("loop"):
        lax.fori_loop(0, 3, outer, 0)

    pL_v, lL_v = (pB_v, lB_v) if (H - 1) % 2 == 1 else (pA_v, lA_v)
    badf = bad_v[...]
    lastl = jnp.concatenate([jnp.sum(lL_v[j], axis=0, keepdims=True) for j in range(NQ)], axis=1)
    badf = jnp.where(lastl >= L_MIN, badf, 1.0)

    is_bad = jnp.max(badf) > 0.5
    for j in range(NQ):
        acc = None
        for cc in range(NC):
            pv = pv_chunk(pL_v, j, cc)
            acc = pv if acc is None else acc + pv
        pv_fin(H - 1, j, acc, lL_v, check=False)

    @pl.when(is_bad)
    def _():
        def fb(h, carry):
            r0 = pl.multiple_of(h * (DH // 2), DH // 2)
            for j in range(NQ):
                cols = pl.ds(j * TQ, TQ)
                qt = _b(jnp.concatenate([qa_v[pl.ds(r0, DH // 2), cols],
                                         jnp.zeros((DH // 2, TQ), U32)], axis=0))

                def sc_(c):
                    k0 = pl.multiple_of(c * (TK // 2), TK // 2)
                    return jnp.dot(_b(ka_v[pl.ds(k0, TK // 2), :]), qt,
                                   preferred_element_type=F32)

                def p1(c, mx):
                    return jnp.maximum(mx, jnp.max(sc_(c).reshape(TK // 8, 8, TQ), axis=0))

                mx = lax.fori_loop(0, NC, p1, jnp.full((8, TQ), -jnp.inf, F32))
                m = jnp.max(mx, axis=0, keepdims=True)

                def p2(c, ls):
                    p = jnp.exp2(sc_(c) - m)
                    k0 = pl.multiple_of(c * (TK // 2), TK // 2)
                    pL_v[pl.ds(k0, TK // 2), cols] = _u(p.astype(BF16))
                    return ls + jnp.sum(p.reshape(TK // 8, 8, TQ), axis=0)

                lL_v[j] = lax.fori_loop(0, NC, p2, jnp.zeros((8, TQ), F32))
                acc = jnp.dot(_b(vT_v[...]), _b(pL_v[:, cols]), preferred_element_type=F32)
                pv_fin(h, j, acc, lL_v, check=False)
            return carry

        lax.fori_loop(0, H, fb, 0)

    wait(cp_modB, 'modB')
    wait(cp_win, 'win')
    wait(cp_wo, 'wo')
    modB = jnp.dot(sc8, wmod_v[...], preferred_element_type=F32)
    ga = modB[0:1, 0:D]
    sb = modB[0:1, D:2 * D]
    cb1 = 1.0 + modB[0:1, 2 * D:3 * D]
    gb = modB[0:1, 3 * D:4 * D]

    def y_blk(e):
        rows = pl.ds(e * TE, TE)
        y = lax.dot_general(_b(oT_v[:, rows]), wo_v[...], (((0,), (0,)), ((), ())),
                            preferred_element_type=F32)
        x1 = x_v[rows, :].astype(F32) + ga * y
        x1_v[rows, :] = x1
        h_v[rows, :] = (_ln(x1) * cb1 + sb).astype(BF16)

    def z2_blk(e):
        rows = pl.ds(e * TE, TE)
        z2 = _gelu_tanh(jnp.dot(h_v[rows, :], win_v[:, pl.ds(FH, FH)], preferred_element_type=F32))
        z2_v[rows, :] = _ln(z2).astype(BF16)

    def z1_blk(e):
        rows = pl.ds(e * TE, TE)
        z1_v[rows, :] = _gelu_tanh(jnp.dot(h_v[rows, :], win_v[:, pl.ds(0, FH)],
                                           preferred_element_type=F32))

    bars = [(cp_bsp, 'bsp'), (cp_wo2, 'b0'), (cp_wout, 'wout'), (cp_wsp, 'wsp')]
    if EBAR == 0:
        for c_, n_ in bars:
            wait(c_, n_)
        bars = []
    y_blk(0)
    for e in range(NE):
        if e + 1 < NE:
            y_blk(e + 1)
        z2_blk(e)
        z1_blk(e)
        if bars and (EBAR == 1 or e == NE - 1):
            wait(*bars.pop(0))
    for c_, n_ in bars:
        wait(c_, n_)

    def out_cp(r):
        return pltpu.make_async_copy(out_v.at[r], out_hbm.at[pl.ds(r * TR, TR), :],
                                     osems.at[r])

    for r in range(NR):
        g = jnp.dot(wsp_v[pl.ds(r * TR, TR), :], z2_v[...], preferred_element_type=F32)
        bcols = []
        for i in range(TR // 128):
            brow = bsp_ref[pl.ds(r * (TR // 128) + i, 1), :].astype(F32)
            bcols.append(jnp.broadcast_to(brow, (128, 128)).T)
        bcol = jnp.concatenate(bcols, axis=0)
        bfull = jnp.concatenate([bcol] * (FH // 128), axis=1)
        u = (z1_v[pl.ds(r * TR, TR), :] * (g + bfull)).astype(BF16)
        yb = jnp.dot(u, wout_v[...], preferred_element_type=F32)
        out_v[r] = (x1_v[pl.ds(r * TR, TR), :] + gb * yb).astype(out_v.dtype)
        out_cp(r).start()
    for r in range(NR):
        wait(out_cp(r), 'out%d' % r)


def make(prof=False, TQ=512, TK=128, XB=(256, 512, 1024), LL=2, TE=512, TR=512, NV=192, G=16, SL=16, EBAR=2, OPQ=False, TCH=2, KB0=6, KB1=14, TKA=5, TL=2, TLU=(2, 3, 6, 7), MSPL=1):
    global PROF
    PROF = prof

    @jax.jit
    def fn(A_x, A_wq, A_wk, A_wv, A_wo, B_x, B_w_in, B_w_sp, B_b_sp, B_w_out, c, w_mod):
        B, S, D = A_x.shape
        DH = A_wk.shape[1]
        H = A_wq.shape[1] // DH
        FH = B_w_in.shape[1] // 2
        NR = S // TR
        NQ = S // TQ
        x2 = A_x.reshape(S, D)
        bsp = B_b_sp.reshape(S // 128, 128)
        any_spec = pl.BlockSpec(memory_space=pl.ANY)
        kern = functools.partial(_kernel, S=S, D=D, H=H, DH=DH, FH=FH,
                                 TQ=TQ, TK=TK, XB=XB, LL=LL, TE=TE, TR=TR, NV=NV, G=G, SL=SL, EBAR=EBAR, OPQ=OPQ,
                                 TCH=TCH, KB0=KB0, KB1=KB1, TKA=TKA, TL=TL, TLU=TLU, MSPL=MSPL)
        out = pl.pallas_call(
            kern,
            out_shape=jax.ShapeDtypeStruct((S, D), A_x.dtype),
            in_specs=[any_spec] * 11,
            out_specs=any_spec,
            scratch_shapes=[
                pltpu.VMEM((S, D), BF16),
                pltpu.VMEM((D, D), BF16),
                pltpu.VMEM((D, D), BF16),
                pltpu.VMEM((D, 2 * FH), BF16),
                pltpu.VMEM((S, S), BF16),
                pltpu.VMEM((FH, D), BF16),
                pltpu.VMEM((D, 4 * D), BF16),
                pltpu.VMEM((D, 2 * D), BF16),
                pltpu.VMEM((D // 2 + DH, D), U32),
                pltpu.VMEM((S, D), BF16),
                pltpu.VMEM((D // 2, S), U32),
                pltpu.VMEM((H, DH, S), F32),
                pltpu.VMEM((S // 128, H, 128), F32),
                pltpu.VMEM((S // 2, 2 * DH), U32),
                pltpu.VMEM((DH, NV, 128), F32),
                pltpu.VMEM((DH // 2, S), U32),
                pltpu.VMEM((S // 2, S), U32),
                pltpu.VMEM((S // 2, S), U32),
                pltpu.VMEM((NQ, 8, TQ), F32),
                pltpu.VMEM((NQ, 8, TQ), F32),
                pltpu.VMEM((NQ, NV, TQ), F32),
                pltpu.VMEM((NQ, NV, TQ), F32),
                pltpu.VMEM((1, S), F32),
                pltpu.VMEM((D // 2, S), U32),
                pltpu.VMEM((S, D), F32),
                pltpu.VMEM((S, FH), F32),
                pltpu.VMEM((S, FH), BF16),
                pltpu.VMEM((NR, TR, D), A_x.dtype),
                pltpu.VMEM((S // 2, D), U32),
                pltpu.VMEM((DH, D), BF16),
                pltpu.VMEM((DH, D), BF16),
                pltpu.VMEM((S // 128, 128), BF16),
                pltpu.VMEM((1, D), BF16),
                pltpu.SemaphoreType.DMA((6 + len(XB) + 1 + 6 + 4,)),
                pltpu.SemaphoreType.DMA((NR,)),
            ],
            compiler_params=pltpu.CompilerParams(vmem_limit_bytes=110 * 1024 * 1024),
            name="fused_block",
        )(x2, A_wq, A_wk.T, A_wv.T, A_wo, B_w_in, B_w_sp, bsp, B_w_out, c, w_mod)
        return out.reshape(B, S, D)
    return fn


_FN = make()


@jax.jit
def pallas_adaLN_cond__grouped_kv_mqa__mixer_gmlp__prompt_kernel(
    A_x: jax.Array,
    A_wq: jax.Array,
    A_wk: jax.Array,
    A_wv: jax.Array,
    A_wo: jax.Array,
    B_x: jax.Array,
    B_w_in: jax.Array,
    B_w_sp: jax.Array,
    B_b_sp: jax.Array,
    B_w_out: jax.Array,
    c: jax.Array,
    w_mod: jax.Array,
):
    return _FN(A_x, A_wq, A_wk, A_wv, A_wo, B_x, B_w_in, B_w_sp, B_b_sp, B_w_out, c, w_mod)
```

```python
import functools
import math

import jax
import jax.numpy as jnp
from jax import lax
import jax.experimental.pallas as pl
import jax.experimental.pallas.tpu as pltpu

F32 = jnp.float32
BF16 = jnp.bfloat16
U32 = jnp.uint32
EPS = 1e-5
LOG2E = 1.4426950408889634
L_MIN = 2.0 ** -60


def _ln(x):
    m = jnp.mean(x, axis=-1, keepdims=True)
    xc = x - m
    v = jnp.mean(xc * xc, axis=-1, keepdims=True)
    return xc * lax.rsqrt(v + EPS)


def _gelu_tanh(x):
    c0 = math.sqrt(2.0 / math.pi)
    inner = x * (c0 + (c0 * 0.044715) * (x * x))
    hx = 0.5 * x
    return hx + hx * jnp.tanh(inner)


PROF = False


class _Null:
    def __enter__(self):
        return self

    def __exit__(self, *a):
        return False


def _scope(name):
    return jax.named_scope(name) if PROF else _Null()


def _b(x):
    return pltpu.bitcast(x, BF16)


def _u(x):
    return pltpu.bitcast(x, U32)


def _kernel(x_hbm, wq_hbm, wkT_hbm, wvT_hbm, wo_hbm, win_hbm, wsp_hbm, bsp_hbm,
            wout_hbm, c_hbm, wmod_hbm, out_hbm,
            x_v, wq_v, wo_v, win_v, wsp_v, wout_v, wmod_v, wmA_v,
            wT_v, h_v, qa_v, q32_v, nm_v, ka_v, kb_v, vT_v,
            pA_v, pB_v, lA_v, lB_v, sA_v, sB_v, bad_v, oT_v, x1_v, z1_v, z2_v,
            out_v, hu_v, wkT_v, wvT_v, bsp_ref, c_v, sems, osems,
            *, S, D, H, DH, FH, TQ, TK, XB, LL, TE, TR, NV, G, SL, EBAR, OPQ, TCH, KB0, KB1, TKA, TL, TLU, MSPL, PB, F0, F1, TS, W0, WF, DP, TWO, PVL, ST):
    NQ = S // TQ
    NC = S // TK
    NE = S // TE
    NR = S // TR
    NT = TQ // 128

    def cp(src, dst, i):
        return pltpu.make_async_copy(src, dst, sems.at[i])

    UT = 128
    NU = S // UT
    xb = [0] + list(XB) + [S]
    NX = len(xb) - 1
    NMA = MSPL
    cp_modAs = [cp(wmod_hbm.at[pl.ds(i * D // NMA, D // NMA), pl.ds(0, 2 * D)], wmA_v.at[pl.ds(i * D // NMA, D // NMA), :], 0 if i == 0 else 6 + NX + 5 + i) for i in range(NMA)]
    cp_wq = cp(wq_hbm, wq_v, 1)
    cp_c = cp(c_hbm, c_v, 2)
    cp_wk = cp(wkT_hbm, wkT_v, 3)
    cp_wv = cp(wvT_hbm, wvT_v, 4)
    cp_bsp = cp(bsp_hbm, bsp_ref, 5)
    cp_x = [cp(x_hbm.at[pl.ds(xb[i], xb[i + 1] - xb[i]), :],
               x_v.at[pl.ds(xb[i], xb[i + 1] - xb[i]), :], 6 + i) for i in range(NX)]
    base = 6 + NX
    cp_modB = cp(wmod_hbm.at[:, pl.ds(2 * D, 4 * D)], wmod_v, base)
    cp_wo = cp(wo_hbm, wo_v, base + 1)
    cp_win = cp(win_hbm, win_v, base + 2)
    cp_wout = cp(wout_hbm, wout_v, base + 3)
    cp_wsp = cp(wsp_hbm.at[pl.ds(0, S // 2), :], wsp_v.at[pl.ds(0, S // 2), :], base + 4)
    cp_wo2 = cp(wsp_hbm.at[pl.ds(S // 2, S // 2), :], wsp_v.at[pl.ds(S // 2, S // 2), :], base + 5)

    def wait(c, name):
        with _scope("w_" + name):
            c.wait()

    for c_ in [cp_wq, cp_x[0], cp_c, cp_wk, cp_wv] + cp_modAs + cp_x[1:]:
        c_.start()

    zer = lax.fori_loop(0, 2, lambda i, c: c * i, jnp.int32(1))

    def dd(r0, n):
        return pl.ds(pl.multiple_of(zer * 16 + r0, 8), n) if OPQ else pl.ds(r0, n)

    zer_u = zer.astype(U32)

    def tie(x, vals):
        t = None
        for v in vals:
            w = v if v.dtype == U32 else pltpu.bitcast(v, U32)
            for r in range(w.shape[0] // 8):
                for c in range(w.shape[1] // 128):
                    p = w[r * 8:(r + 1) * 8, c * 128:(c + 1) * 128]
                    t = p if t is None else t | p
        if t is None:
            return x
        top = x[:8, :128] | (t & zer_u)
        if x.shape[1] > 128:
            top = jnp.concatenate([top, x[:8, 128:]], axis=1)
        return jnp.concatenate([top, x[8:]], axis=0)

    bad_v[...] = jnp.zeros(bad_v.shape, F32)
    e_r = lax.broadcasted_iota(jnp.int32, (H, D), 0)
    e_c = lax.broadcasted_iota(jnp.int32, (H, D), 1)
    emat = jnp.where((e_c >= e_r * DH) & (e_c < (e_r + 1) * DH), 1.0, 0.0).astype(BF16)
    aug_r = lax.broadcasted_iota(jnp.int32, (DH, UT), 0)
    aug = jnp.where(aug_r < 2, 1.0, 0.0).astype(F32)
    qscale = (DH ** -0.5) * LOG2E

    wait(cp_wq, 'wq')
    wT_v[pl.ds(0, D // 2), :] = _u(wq_v[...].astype(F32).T.astype(BF16))
    wait(cp_x[0], 'x0')
    x1_v[pl.ds(0, xb[1]), :] = _ln(x_v[pl.ds(0, xb[1]), :].astype(F32))
    wait(cp_c, 'c')
    wait(cp_wk, 'wk')
    wait(cp_wv, 'wv')
    wT_v[pl.ds(D // 2, DH // 2), :] = _u(wvT_v[...])
    wT_v[pl.ds((D + DH) // 2, DH // 2), :] = _u(wkT_v[...])
    cvec = c_v[...].astype(F32)
    sc = cvec * (1.0 / (1.0 + jnp.exp(-cvec)))
    sc8 = jnp.broadcast_to(sc, (8, D)).astype(BF16)

    for c_ in cp_modAs:
        wait(c_, 'modA')
    modA = jnp.dot(sc8, wmA_v[...], preferred_element_type=F32)
    sa = modA[0:1, 0:D]
    ca1 = 1.0 + modA[0:1, D:2 * D]

    def ln1(r0, n):
        if r0 < xb[1]:
            xh = x1_v[dd(r0, n), :]
        else:
            xh = _ln(x_v[pl.ds(r0, n), :].astype(F32))
        hv = _u((xh * ca1 + sa).astype(BF16))
        hu_v[pl.ds(r0 // 2, n // 2), :] = hv
        return hv

    kst = {}
    NT_ = (((1,), (1,)), ((), ()))

    kbd = {}
    for d in range(DH):
        kbd.setdefault(KB0 + d * (KB1 - KB0) // DH, []).append(d)

    def norms(u):
        qn2 = jnp.dot(emat, jnp.concatenate(kst.pop(u), axis=0), preferred_element_type=F32)
        qn = jnp.sqrt(qn2)
        for hh in range(H):
            nm_v[hh, pl.ds(u // 2, 1), pl.ds(u % 2 * 128, 128)] = qn[hh:hh + 1]

    def qkv(u):
        sq = kst[u] = []
        cols = pl.ds(u * UT, UT)
        hb = _b(hu_v[dd(u * UT // 2, UT // 2), :])
        un = u + LL
        nch = D // 128
        for ch in range(nch):
            last = ch == nch - 1
            nrow = 128 + (2 * DH if last else 0)
            wch = wT_v[dd(ch * 64, nrow // 2), :]
            tl = kst.pop(('ln', u * nch + ch), [])
            if ch == TCH:
                tl = tl + kst.pop('tie', [])
            wch = tie(wch, tl)
            qv = lax.dot_general(_b(wch), hb, NT_,
                                 preferred_element_type=F32)
            qs = qv[:128] * qscale
            qa_v[pl.ds(ch * 64, 64), cols] = _u(qs.astype(BF16))
            q32_v[pl.ds(ch * 8, 8), :, cols] = qs.reshape(8, DH, UT)
            sq.append((qs * qs).astype(BF16))
            if ch == 1 and u > 0:
                norms(u - 1)
            if last:
                vT_v[:, cols] = _u(qv[128:128 + DH].astype(BF16))
                kT = qv[128 + DH:]
                k2 = jnp.sum(kT * kT, axis=0, keepdims=True)
                kst['k2'] = k2 if u == 0 else jnp.maximum(kst['k2'], k2)
                kaug = jnp.concatenate([kT, aug], axis=0).T
                kau = _u(kaug.astype(BF16))
                ka_v[pl.ds(u * UT // 2, UT // 2), :] = kau
                nkb = min(UT, NV - u * UT)
                if nkb > 0:
                    kst.setdefault('kf', []).append(kaug[:nkb])
                if TKA:
                    kst.setdefault(('ln', (u + 1) * nch + TKA), []).append(
                        jnp.concatenate([kau, jnp.zeros((UT // 2, 128 - 2 * DH), U32)], axis=1))
                tv = []
                for d in kbd.get(u, []):
                    kf = jnp.concatenate(kst['kf'], axis=0)
                    kbv = jnp.broadcast_to(kf[:, d:d + 1], (NV, 128))
                    kb_v[d] = kbv
                    tv.append(kbv)
                kst['tie'] = tv
            if un < NU:
                hv = ln1(un * UT + ch * (UT // nch), UT // nch)
                if TL and un in TLU:
                    kst.setdefault(('ln', u * nch + ch + TL), []).append(hv)

    nx = 1
    for u in range(NU):
        need = min(u + LL + 1, NU) * UT
        while nx < NX and xb[nx] < need:
            wait(cp_x[nx], 'x%d' % nx)
            nx += 1
        if u == 0:
            for v in range(LL):
                ln1(v * UT, UT)
        qkv(u)
    norms(NU - 1)

    kmax = jnp.sqrt(jnp.max(kst['k2'], axis=1, keepdims=True)) * (-1.015625)
    for hh in range(H):
        nm_v[hh] = (nm_v[hh] * kmax).astype(BF16).astype(F32)

    def nm_row(h, c0):
        return nm_v[h, pl.ds(c0 // 256, 1), pl.ds(c0 % 256, 128)]

    def q_tile(h, j):
        r0 = h * (DH // 2) if isinstance(h, int) else pl.multiple_of(h * (DH // 2), DH // 2)
        q = qa_v[pl.ds(r0, DH // 2), pl.ds(j * TQ, TQ)]
        m = jnp.concatenate(
            [jnp.broadcast_to(nm_row(h, j * TQ + t * 128), (DH // 2, 128)) for t in range(NT)],
            axis=1)
        return _b(jnp.concatenate([q, pltpu.bitcast(m, U32)], axis=0))

    class Piece:
        def __init__(s, h, j, g, w):
            s.h, s.j, s.g, s.w = h, j, g, w
            s.a = None
            s.d = 0

        def step(s):
            c0 = [s.j * TQ + t * 128 for t in range(NT)]
            if s.a is None:
                s.a = [jnp.broadcast_to(nm_row(s.h, c0[t]), (G, 128)) for t in range(NT)]
            kb = kb_v[s.d, pl.ds(s.g * G, G), :]
            for t in range(NT):
                s.a[t] = s.a[t] + kb * q32_v[s.h, pl.ds(s.d, 1), pl.ds(c0[t], 128)]
            s.d += 1
            return s.a

        def fin(s):
            s.w[s.j, pl.ds(s.g * G, G), :] = jnp.concatenate(s.a, axis=1)
            return None

    def never(n):
        return lax.broadcasted_iota(jnp.int32, (8, n), 1) < zer

    def pv_chunk(p_r, j, cc, f=lambda x: x[...]):
        pb = _b(p_r[pl.ds(cc * TK // 2, TK // 2), pl.ds(j * TQ, TQ)])
        return jnp.dot(_b(f(vT_v.at[:, pl.ds(cc * TK, TK)])), pb, preferred_element_type=F32)

    def pv_fin(hp, j, acc, l_r, check=True):
        cols = pl.ds(j * TQ, TQ)
        l = jnp.sum(l_r[j], axis=0, keepdims=True)
        r0 = hp * (DH // 2) if isinstance(hp, int) else pl.multiple_of(hp * (DH // 2), DH // 2)
        oT_v[pl.ds(r0, DH // 2), cols] = _u((acc * (1.0 / l)).astype(BF16))
        if check:
            bad_v[:, cols] = jnp.where(l >= L_MIN, bad_v[:, cols], 1.0)

    def region(parts, last=False):
        stream, done = [], {}
        plan, room = [], [W0] * F0
        for pi, (h, p_r, l_r, p_w, l_w, s_r, s_w) in enumerate(parts):
            first = s_r is None
            k0 = 0 if first else NV
            if not last:
                for j in range(NQ):
                    for g in range(NV // G):
                        pc = Piece(h + 1, j, g, s_w)
                        stream += [pc.step] * DH + [pc.fin]
                        done[(pi + 1, j, g)] = len(stream)
            ns = (S - k0) // SL
            cut = [c * ns // NC for c in range(NC + 1)]
            for j in range(NQ):
                raws = [] if first else list(range(0, NV, SL))
                pvs = [] if first else [(0, j, cc) for cc in range(NC)]
                if last and j > 0:
                    own = [(1, j - 1, cc) for cc in range(NC)]
                    pvs = [x for y in zip(pvs, own) for x in y]
                nr, npv = len(raws), len(pvs)
                c0 = DP if (pi > 0 and j == 0) else 0
                for c in range(NC):
                    plan.append(('dot', pi, j, k0 + cut[c] * SL, k0 + cut[c + 1] * SL))
                    room += [43] * (cut[c + 1] - cut[c])
                    debt = 0
                    while len(raws) > nr - -(-(c + 1 - c0) * nr // (NC - c0)):
                        plan.append(('raw', pi, j, raws.pop(0)))
                        debt += 20
                    while len(pvs) > npv - -(-(c + 1 - c0) * npv // (NC - c0)):
                        plan.append(('pv', pi) + pvs.pop(0))
                        room.append(55 - debt)
                        debt = 0
                    room[-1] -= debt
                plan.append(('fin', pi, j))
                if not first:
                    room[-1] -= WF
        room = room[:len(room) + F1]
        cum = []
        for w in room:
            cum.append(w + (cum[-1] if cum else 0))
        gs = dict(n=-F0, up={}, i=0, l=None)
        acc = [None, None]

        def emit_fma():
            n = gs['n']
            tgt = len(stream) if n + F0 >= len(cum) else -(-cum[n + F0] * len(stream) // cum[-1])
            while gs['i'] < min(tgt, len(stream)):
                a = stream[gs['i']]()
                gs['i'] += 1
                if a is not None:
                    w = (n * TS) % (NT * G // 8)
                    gs['up'][n + PB] = a[w % NT][(w // NT) * 8:(w // NT) * 8 + 8]
            gs['n'] += 1

        def tied(ref, n):
            up = gs['up'].pop(n, None)
            if up is None:
                return ref[...]
            w = ref.shape[1]
            up = pltpu.bitcast(up, U32)[:, :w]
            if ST:
                pltpu.store(ref, up, mask=never(w))
                return ref[...]
            return jnp.where(never(w), up, ref[...])

        def slabs(s, p_w, j, row0, n, emit):
            for r in range(n // SL):
                p = jnp.exp2(s[r * SL:(r + 1) * SL])
                cs = jnp.sum(p.reshape(SL // 8, 8, TQ), axis=0)
                gs['l'] = cs if gs['l'] is None else gs['l'] + cs
                p_w[pl.ds((row0 + r * SL) // 2, SL // 2), pl.ds(j * TQ, TQ)] = _u(p.astype(BF16))
                if emit:
                    emit_fma()

        while gs['n'] < 0:
            emit_fma()
        for ev in plan:
            h, p_r, l_r, p_w, l_w, s_r, s_w = parts[ev[1]]
            j = ev[2]
            if ev[0] == 'dot':
                lo, hi = ev[3:]
                ka = jnp.concatenate([tied(ka_v.at[pl.ds(lo // 2 + r * 8, 8), :], gs['n'] + r)
                                      for r in range((hi - lo) // SL)], axis=0)
                s = jnp.dot(_b(ka), q_tile(h, j), preferred_element_type=F32)
                slabs(s, p_w, j, lo, hi - lo, True)
            elif ev[0] == 'raw':
                assert ev[1] == 0 or done[(ev[1], j, ev[3] // G)] <= gs['i']
                slabs(s_r[j + zer if ev[1] else j, pl.ds(ev[3], SL), :], p_w, j, ev[3], SL, False)
            elif ev[0] == 'pv':
                o, jj, cc = ev[2:]
                pv = pv_chunk(p_w if o else p_r, jj, cc, lambda x: tied(x, gs['n']))
                acc[o] = pv if acc[o] is None else acc[o] + pv
                emit_fma()
            else:
                l_w[j] = gs['l']
                if acc[0] is not None:
                    pv_fin(h - 1, j, acc[0], l_r)
                if acc[1] is not None:
                    pv_fin(h, j - 1, acc[1], l_w, check=False)
                gs['l'] = acc[0] = acc[1] = None
        assert gs['i'] == len(stream)

    def odd(h):
        return (h, pA_v, lA_v, pB_v, lB_v, sB_v, sA_v)

    def even(h):
        return (h, pB_v, lB_v, pA_v, lA_v, sA_v, sB_v)

    def pair(i, carry):
        if TWO:
            region([odd(2 * i + 1), even(2 * i + 2)])
        else:
            @pl.when(i >= 0)
            def _():
                region([odd(2 * i + 1)])

            @pl.when(i < H)
            def _():
                region([even(2 * i + 2)])

        return carry

    def outer(t, carry):
        @pl.when(t == 0)
        def _():
            region([(t, None, None, pA_v, lA_v, None, sB_v)])

        @pl.when(t == 2)
        def _():
            for c_ in [cp_wo, cp_modB, cp_win, cp_wout, cp_wsp, cp_wo2, cp_bsp]:
                c_.start()

        @pl.when(t >= 1)
        def _():
            lax.fori_loop(t - 1, jnp.where(t == 1, 1, H // 2 - 1), pair, 0)

        return carry

    with _scope("loop"):
        lax.fori_loop(0, 3, outer, 0)

    assert H % 2 == 0
    region([odd(H - 1)], last=True)
    pL_v, lL_v = pB_v, lB_v
    badf = bad_v[...]
    lastl = jnp.concatenate([jnp.sum(lL_v[j], axis=0, keepdims=True) for j in range(NQ)], axis=1)
    badf = jnp.where(lastl >= L_MIN, badf, 1.0)
    is_bad = jnp.max(badf) > 0.5

    def pv_last():
        acc = None
        for cc in range(NC):
            pv = pv_chunk(pL_v, NQ - 1, cc)
            acc = pv if acc is None else acc + pv
        pv_fin(H - 1, NQ - 1, acc, lL_v, check=False)

    if PVL < 0:
        pv_last()

    @pl.when(is_bad)
    def _():
        def fb(h, carry):
            r0 = pl.multiple_of(h * (DH // 2), DH // 2)
            for j in range(NQ):
                cols = pl.ds(j * TQ, TQ)
                qt = _b(jnp.concatenate([qa_v[pl.ds(r0, DH // 2), cols],
                                         jnp.zeros((DH // 2, TQ), U32)], axis=0))

                def sc_(c):
                    k0 = pl.multiple_of(c * (TK // 2), TK // 2)
                    return jnp.dot(_b(ka_v[pl.ds(k0, TK // 2), :]), qt,
                                   preferred_element_type=F32)

                def p1(c, mx):
                    return jnp.maximum(mx, jnp.max(sc_(c).reshape(TK // 8, 8, TQ), axis=0))

                mx = lax.fori_loop(0, NC, p1, jnp.full((8, TQ), -jnp.inf, F32))
                m = jnp.max(mx, axis=0, keepdims=True)

                def p2(c, ls):
                    p = jnp.exp2(sc_(c) - m)
                    k0 = pl.multiple_of(c * (TK // 2), TK // 2)
                    pL_v[pl.ds(k0, TK // 2), cols] = _u(p.astype(BF16))
                    return ls + jnp.sum(p.reshape(TK // 8, 8, TQ), axis=0)

                lL_v[j] = lax.fori_loop(0, NC, p2, jnp.zeros((8, TQ), F32))
                acc = jnp.dot(_b(vT_v[...]), _b(pL_v[:, cols]), preferred_element_type=F32)
                pv_fin(h, j, acc, lL_v, check=False)
            return carry

        lax.fori_loop(0, H, fb, 0)

    wait(cp_modB, 'modB')
    wait(cp_win, 'win')
    wait(cp_wo, 'wo')
    modB = jnp.dot(sc8, wmod_v[...], preferred_element_type=F32)
    ga = modB[0:1, 0:D]
    sb = modB[0:1, D:2 * D]
    cb1 = 1.0 + modB[0:1, 2 * D:3 * D]
    gb = modB[0:1, 3 * D:4 * D]

    def y_blk(e):
        rows = pl.ds(e * TE, TE)
        y = lax.dot_general(_b(oT_v[:, rows]), wo_v[...], (((0,), (0,)), ((), ())),
                            preferred_element_type=F32)
        x1 = x_v[rows, :].astype(F32) + ga * y
        x1_v[rows, :] = x1
        h_v[rows, :] = (_ln(x1) * cb1 + sb).astype(BF16)

    def z2_blk(e):
        rows = pl.ds(e * TE, TE)
        z2 = _gelu_tanh(jnp.dot(h_v[rows, :], win_v[:, pl.ds(FH, FH)], preferred_element_type=F32))
        z2_v[rows, :] = _ln(z2).astype(BF16)

    def z1_blk(e):
        rows = pl.ds(e * TE, TE)
        z1_v[rows, :] = _gelu_tanh(jnp.dot(h_v[rows, :], win_v[:, pl.ds(0, FH)],
                                           preferred_element_type=F32))

    bars = [(cp_bsp, 'bsp'), (cp_wo2, 'b0'), (cp_wout, 'wout'), (cp_wsp, 'wsp')]
    if EBAR == 0:
        for c_, n_ in bars:
            wait(c_, n_)
        bars = []
    y_blk(0)
    for e in range(NE):
        if e == PVL:
            pv_last()
        if e + 1 < NE:
            y_blk(e + 1)
        z2_blk(e)
        z1_blk(e)
        if bars and (EBAR == 1 or e == NE - 1):
            wait(*bars.pop(0))
    for c_, n_ in bars:
        wait(c_, n_)

    def out_cp(r):
        return pltpu.make_async_copy(out_v.at[r], out_hbm.at[pl.ds(r * TR, TR), :],
                                     osems.at[r])

    for r in range(NR):
        g = jnp.dot(wsp_v[pl.ds(r * TR, TR), :], z2_v[...], preferred_element_type=F32)
        bcols = []
        for i in range(TR // 128):
            brow = bsp_ref[pl.ds(r * (TR // 128) + i, 1), :].astype(F32)
            bcols.append(jnp.broadcast_to(brow, (128, 128)).T)
        bcol = jnp.concatenate(bcols, axis=0)
        bfull = jnp.concatenate([bcol] * (FH // 128), axis=1)
        u = (z1_v[pl.ds(r * TR, TR), :] * (g + bfull)).astype(BF16)
        yb = jnp.dot(u, wout_v[...], preferred_element_type=F32)
        out_v[r] = (x1_v[pl.ds(r * TR, TR), :] + gb * yb).astype(out_v.dtype)
        out_cp(r).start()
    for r in range(NR):
        wait(out_cp(r), 'out%d' % r)


def make(prof=False, TQ=512, TK=128, XB=(256, 512, 1024), LL=2, TE=512, TR=512, NV=304, G=16, SL=16, EBAR=2, OPQ=False, TCH=2, KB0=6, KB1=14, TKA=5, TL=2, TLU=(2, 3, 6, 7), MSPL=1, PB=8, F0=7, F1=-8, TS=3, W0=55, WF=150, DP=2, TWO=False, PVL=-1, ST=False):
    global PROF
    PROF = prof

    @jax.jit
    def fn(A_x, A_wq, A_wk, A_wv, A_wo, B_x, B_w_in, B_w_sp, B_b_sp, B_w_out, c, w_mod):
        B, S, D = A_x.shape
        DH = A_wk.shape[1]
        H = A_wq.shape[1] // DH
        FH = B_w_in.shape[1] // 2
        NR = S // TR
        NQ = S // TQ
        x2 = A_x.reshape(S, D)
        bsp = B_b_sp.reshape(S // 128, 128)
        any_spec = pl.BlockSpec(memory_space=pl.ANY)
        kern = functools.partial(_kernel, S=S, D=D, H=H, DH=DH, FH=FH,
                                 TQ=TQ, TK=TK, XB=XB, LL=LL, TE=TE, TR=TR, NV=NV, G=G, SL=SL, EBAR=EBAR, OPQ=OPQ,
                                 TCH=TCH, KB0=KB0, KB1=KB1, TKA=TKA, TL=TL, TLU=TLU, MSPL=MSPL, PB=PB, F0=F0, F1=F1, TS=TS, W0=W0, WF=WF, DP=DP, TWO=TWO, PVL=PVL, ST=ST)
        out = pl.pallas_call(
            kern,
            out_shape=jax.ShapeDtypeStruct((S, D), A_x.dtype),
            in_specs=[any_spec] * 11,
            out_specs=any_spec,
            scratch_shapes=[
                pltpu.VMEM((S, D), BF16),
                pltpu.VMEM((D, D), BF16),
                pltpu.VMEM((D, D), BF16),
                pltpu.VMEM((D, 2 * FH), BF16),
                pltpu.VMEM((S, S), BF16),
                pltpu.VMEM((FH, D), BF16),
                pltpu.VMEM((D, 4 * D), BF16),
                pltpu.VMEM((D, 2 * D), BF16),
                pltpu.VMEM((D // 2 + DH, D), U32),
                pltpu.VMEM((S, D), BF16),
                pltpu.VMEM((D // 2, S), U32),
                pltpu.VMEM((H, DH, S), F32),
                pltpu.VMEM((H, S // 256, 256), F32),
                pltpu.VMEM((S // 2, 2 * DH), U32),
                pltpu.VMEM((DH, NV, 128), F32),
                pltpu.VMEM((DH // 2, S), U32),
                pltpu.VMEM((S // 2, S), U32),
                pltpu.VMEM((S // 2, S), U32),
                pltpu.VMEM((NQ, 8, TQ), F32),
                pltpu.VMEM((NQ, 8, TQ), F32),
                pltpu.VMEM((NQ, NV, TQ), F32),
                pltpu.VMEM((NQ, NV, TQ), F32),
                pltpu.VMEM((1, S), F32),
                pltpu.VMEM((D // 2, S), U32),
                pltpu.VMEM((S, D), F32),
                pltpu.VMEM((S, FH), F32),
                pltpu.VMEM((S, FH), BF16),
                pltpu.VMEM((NR, TR, D), A_x.dtype),
                pltpu.VMEM((S // 2, D), U32),
                pltpu.VMEM((DH, D), BF16),
                pltpu.VMEM((DH, D), BF16),
                pltpu.VMEM((S // 128, 128), BF16),
                pltpu.VMEM((1, D), BF16),
                pltpu.SemaphoreType.DMA((6 + len(XB) + 1 + 6 + 4,)),
                pltpu.SemaphoreType.DMA((NR,)),
            ],
            compiler_params=pltpu.CompilerParams(vmem_limit_bytes=110 * 1024 * 1024),
            name="fused_block",
        )(x2, A_wq, A_wk.T, A_wv.T, A_wo, B_w_in, B_w_sp, bsp, B_w_out, c, w_mod)
        return out.reshape(B, S, D)
    return fn


_FN = make()


@jax.jit
def pallas_adaLN_cond__grouped_kv_mqa__mixer_gmlp__prompt_kernel(
    A_x: jax.Array,
    A_wq: jax.Array,
    A_wk: jax.Array,
    A_wv: jax.Array,
    A_wo: jax.Array,
    B_x: jax.Array,
    B_w_in: jax.Array,
    B_w_sp: jax.Array,
    B_b_sp: jax.Array,
    B_w_out: jax.Array,
    c: jax.Array,
    w_mod: jax.Array,
):
    return _FN(A_x, A_wq, A_wk, A_wv, A_wo, B_x, B_w_in, B_w_sp, B_b_sp, B_w_out, c, w_mod)
```
